```python
import os as _os
_os.environ.setdefault("JAX_PLATFORMS", "cpu")
import jax
import jax.numpy as jnp

def _softmax(x, axis=-1):
    return jax.nn.softmax(x, axis=axis)
def _gelu(x):
    return jax.nn.gelu(x, approximate=True)
def _silu(x):
    return jax.nn.silu(x)
def _sigmoid(x):
    return jax.nn.sigmoid(x)
def _layernorm(x, axis=-1, eps=1e-5):
    m = jnp.mean(x, axis=axis, keepdims=True)
    v = jnp.var(x, axis=axis, keepdims=True)
    return (x - m) / jnp.sqrt(v + eps)
def _scatter_add(tgt, idx, src, axis=0):
    return tgt.at[idx].add(src)
def _segment_sum(src, seg, n):
    return jax.ops.segment_sum(src, seg, n)
class _Rng:
    def __init__(self, key):
        self._k = key
    def _next(self):
        self._k, sub = jax.random.split(self._k)
        return sub
    def normal(self, shape):
        return jax.random.normal(self._next(), shape, dtype=jnp.bfloat16)
    def randint(self, lo, hi, shape):
        return jax.random.randint(self._next(), shape, lo, hi, dtype=jnp.int32)
    def uniform(self, shape, lo=0.0, hi=1.0):
        return jax.random.uniform(self._next(), shape, jnp.bfloat16, lo, hi)
    def permutation(self, n):
        return jax.random.permutation(self._next(), n)


kernel_name = 'concat_heads__mha_block__linear_attn_block__prompt'

def setup_inputs():
    _rng = _Rng(jax.random.key(int.from_bytes(__import__("os").urandom(4), "little")))
    _w = (lambda a: (lambda t: t.astype(jnp.bfloat16) if jnp.issubdtype(t.dtype, jnp.floating) else t)(jnp.asarray(a)))
    def _A_setup():
        B, S, D, H = 1, 2048, 1024, 32
        return {
            "x": _w((lambda *s: _rng.normal(s) * 0.2)(B, S, D)),
            "wqkv": _w((lambda *s: _rng.normal(s) * 0.2)(D, 3 * D)),
            "wo": _w((lambda *s: _rng.normal(s) * 0.05)(D, D)),
        }
    _A_in = _A_setup()

    def _B_setup():
        B, S, D = 1, 2048, 1024
        return {
            "x": _w((lambda *s: _rng.normal(s) * 0.05)(B, S, D)),
            "wqkv": _w((lambda *s: _rng.normal(s) * 1.6)(D, 3 * D)),
            "wo": _w((lambda *s: _rng.normal(s) * 0.1)(D, D)),
        }
    _B_in = _B_setup()

    return {
        "A_x": _A_in["x"],
        "A_wqkv": _A_in["wqkv"],
        "A_wo": _A_in["wo"],
        "B_x": _B_in["x"],
        "B_wqkv": _B_in["wqkv"],
        "B_wo": _B_in["wo"],
    }

def reference(A_x, A_wqkv, A_wo, B_x, B_wqkv, B_wo):
    def _A_ref(x, wqkv, wo):
        B, S, D = x.shape
        H = 32
        Dh = D // H
        qkv = (lambda x, *d: x.transpose(*d))((x @ wqkv).reshape(B, S, 3, H, Dh), 2, 0, 3, 1, 4)
        q, k, v = qkv[0], qkv[1], qkv[2]
        scores = jnp.einsum("bhqd,bhkd->bhqk", q, k) * (Dh ** -0.5)
        p = _softmax(scores, axis=-1)
        o = jnp.einsum("bhqk,bhkd->bhqd", p, v)
        return (lambda x, *d: x.transpose(*d))(o, 0, 2, 1, 3).reshape(B, S, D) @ wo

    def _B_ref(x, wqkv, wo):
        B, S, D = x.shape
        H = 32; Dh = D // H
        qkv = (lambda x, *d: x.transpose(*d))((x @ wqkv).reshape(B, S, 3, H, Dh), 2, 0, 3, 1, 4)
        q, k, v = qkv[0], qkv[1], qkv[2]
        phi = lambda t: jnp.where(t > 0, t + 1, jnp.exp(t)) + 1e-6
        pq, pk = phi(q), phi(k)
        kv = jnp.einsum("bhsd,bhse->bhde", pk, v)
        z = jnp.einsum("bhsd->bhd", pk)
        num = jnp.einsum("bhqd,bhde->bhqe", pq, kv)
        den = jnp.einsum("bhqd,bhd->bhq", pq, z)[..., None] + 1e-6
        o = num / den
        return (lambda x, *d: x.transpose(*d))(o, 0, 2, 1, 3).reshape(B, S, D) @ wo

    a = _A_ref(A_x, A_wqkv, A_wo)
    b = _B_ref(B_x, B_wqkv, B_wo)
    return jnp.concatenate([a, b], axis=-1)
```

```python
import math

import jax
import jax.numpy as jnp
from jax import lax
import jax.experimental.pallas as pl
import jax.experimental.pallas.tpu as pltpu

f32 = jnp.float32
bf16 = jnp.bfloat16

S = 2048
D = 1024
H = 32
DH = D // H
G = 128 // DH
NG = D // 128

TQ = 512
CK = 256
SUB = 32
SK = 1
UN = G
NQ = S // TQ
NU = H * NQ
NC = S // CK
NS = CK // SUB

NT = (((1,), (1,)), ((), ()))
TN = (((0,), (0,)), ((), ()))

QSCALE = (DH ** -0.5) * math.log2(math.e)


def _phi(t):
    return jnp.where(t > 0, t + 1.0, jnp.exp(t)) + 1e-6


def _kernel(xa_hbm, wa_hbm, woa_hbm, xb_hbm, wb_hbm, wob_hbm, out_hbm,
            xa, wa, woa, xb, wb, wob,
            k_s, qt_s, vt_s, ot_s, sa, sb, kv_s, z_s, m_s, oa_st, ob_st,
            in_sem, out_sem):
    in_copies = []

    def add_in(src, dst):
        cp = pltpu.make_async_copy(src, dst, in_sem.at[len(in_copies)])
        in_copies.append(cp)
        return cp

    XR = 512
    c_xa = [add_in(xa_hbm.at[pl.ds(i * XR, XR), :], xa.at[pl.ds(i * XR, XR), :]) for i in range(S // XR)]
    c_wa = [add_in(wa_hbm.at[:, pl.ds(j * D, D)], wa.at[:, pl.ds(j * D, D)]) for j in range(3)]
    c_woa = add_in(woa_hbm, woa)
    c_xb = add_in(xb_hbm, xb)
    c_wb = add_in(wb_hbm, wb)
    c_wob = add_in(wob_hbm, wob)

    c_xa[0].start()
    c_wa[1].start()
    for i in range(1, S // XR):
        c_xa[i].start()

    c_wa[1].wait()
    for i in range(S // XR):
        c_xa[i].wait()
        if i == 0:
            c_wa[0].start()
            c_wa[2].start()
        y = jnp.dot(xa[i * XR:(i + 1) * XR, :], wa[:, D:2 * D], preferred_element_type=f32)
        k_s[i * XR:(i + 1) * XR, :] = y.astype(bf16)

    c_wa[0].wait()
    c_wa[2].wait()
    c_woa.start()
    c_xb.start()
    c_wb.start()
    c_wob.start()

    WC = 512

    def qv_body(j, carry):
        half = D // WC
        is_v = j // half
        co = pl.multiple_of((j % half) * WC, WC)
        wco = pl.multiple_of(is_v * (2 * D) + co, WC)
        wt = wa[:, pl.ds(wco, WC)].astype(f32).T.astype(bf16)
        scale = jnp.where(is_v == 0, QSCALE, 1.0).astype(f32)
        for i in range(2):
            r = S // 2
            y = lax.dot_general(wt, xa[i * r:(i + 1) * r, :], NT, preferred_element_type=f32)
            qv_t[is_v, pl.ds(co, WC), i * r:(i + 1) * r] = (y * scale).astype(bf16)
        return carry

    qv_t = qt_s
    lax.fori_loop(0, 2 * (D // WC), qv_body, 0)

    bufs = (sa, sb)

    def q_weights(u, hh):
        h = u % H
        qi = u // H
        goff = pl.multiple_of((h // G) * 128, 128)
        hoff = pl.multiple_of(h * DH, DH)
        qoff = pl.multiple_of(qi * TQ, TQ)
        qh = qv_t[0, pl.ds(hoff, DH), pl.ds(qoff, TQ)]
        parts = []
        if hh > 0:
            parts.append(jnp.zeros((hh * DH, TQ), bf16))
        parts.append(qh)
        if hh < G - 1:
            parts.append(jnp.zeros(((G - 1 - hh) * DH, TQ), bf16))
        return goff, jnp.concatenate(parts, axis=0)

    def run(base, a_slots, c_slots, m_known, mp):
        qms = {}
        prev_mh = None
        acc = None
        lhist = []
        for a, cc in zip(a_slots, c_slots):
            mh = None
            if a is not None:
                ua, c = a
                if ua not in qms:
                    u = base + ua
                    u = jnp.where(u < NU, u, u - G)
                    qms[ua] = q_weights(u, ua % G)
                goff, qm = qms[ua]
                kg = k_s[c * CK:(c + 1) * CK, pl.ds(goff, 128)]
                s = jnp.dot(kg, qm, preferred_element_type=f32)
                bufs[ua % 2][c * CK:(c + 1) * CK, :] = s
                mh = []
                for j in range(NS):
                    sm = jnp.max(s[j * SUB:(j + 1) * SUB].reshape(SUB // 8, 8, TQ), axis=0)
                    mp = sm if (c == 0 and j == 0) else jnp.maximum(mp, sm)
                    mh.append(mp)
                if c == NC - 1:
                    m_known[ua] = jnp.max(mp, axis=0, keepdims=True)
            if cc is not None:
                uc, c = cc
                u = base + uc
                h = u % H
                qi = u // H
                hoff = pl.multiple_of(h * DH, DH)
                qoff = pl.multiple_of(qi * TQ, TQ)
                s_c = bufs[uc % 2]
                m_c = m_known[uc]
                if c == 0:
                    lhist = []
                ps_ = []
                for j in range(NS):
                    g = c * NS + j
                    r0 = c * CK + j * SUB
                    d0 = s_c[r0:r0 + 8, :] - m_c
                    if g >= 1:
                        d0 = jnp.minimum(d0, lhist[g - 1])
                    if prev_mh is not None:
                        d0 = jnp.minimum(d0, jnp.abs(prev_mh[j]))
                    d1 = s_c[r0 + 8:r0 + SUB, :] - m_c
                    p = jnp.exp2(jnp.concatenate([d0, d1], axis=0))
                    ps = jnp.sum(p.reshape(SUB // 8, 8, TQ), axis=0)
                    lhist.append(ps if g == 0 else lhist[-1] + ps)
                    ps_.append(p)
                pb = jnp.concatenate(ps_, axis=0).astype(bf16)
                vt = qv_t[1, pl.ds(hoff, DH), c * CK:(c + 1) * CK]
                o = jnp.dot(vt, pb, preferred_element_type=f32)
                acc = o if c == 0 else acc + o
                if c == NC - 1:
                    l = jnp.sum(lhist[-1], axis=0, keepdims=True)
                    ot_s[pl.ds(hoff, DH), pl.ds(qoff, TQ)] = (acc * (1.0 / l)).astype(bf16)
            prev_mh = mh
        return m_known, mp

    a0 = [(t // NC, t % NC) for t in range(NC + SK)]
    mk, mp0 = run(0, a0, [None] * len(a0), {}, None)

    def att_body(i, carry):
        m0, mp = carry
        n = UN * NC
        a = [((t + NC + SK) // NC, (t + NC + SK) % NC) for t in range(n)]
        c = [(t // NC, t % NC) for t in range(n)]
        mk_, mp = run(i * UN, a, c, {0: m0}, mp)
        return mk_[UN], mp

    lax.fori_loop(0, NU // UN, att_body, (mk[0], mp0))

    OR = 512
    n_or = S // OR

    def out_copy(st, blk, col, sem_idx):
        ro = pl.multiple_of(blk * OR, OR)
        return pltpu.make_async_copy(
            st.at[pl.ds(ro, OR), :], out_hbm.at[pl.ds(ro, OR), pl.ds(col, D)], out_sem.at[sem_idx])

    c_woa.wait()

    def oa_body(i, carry):
        ro = pl.multiple_of(i * OR, OR)
        y = lax.dot_general(ot_s[:, pl.ds(ro, OR)], woa[...], TN, preferred_element_type=f32)
        oa_st[pl.ds(ro, OR), :] = y.astype(bf16)
        out_copy(oa_st, i, 0, i).start()
        return carry

    lax.fori_loop(0, n_or, oa_body, 0)

    c_xb.wait()
    c_wb.wait()
    c_wob.wait()

    kv_s[...] = jnp.zeros_like(kv_s)
    z_s[...] = jnp.zeros_like(z_s)
    BR = 512

    def bkv_body(i, carry):
        ro = pl.multiple_of(i * BR, BR)
        xblk = xb[pl.ds(ro, BR), :]
        pk = _phi(jnp.dot(xblk, wb[:, D:2 * D], preferred_element_type=f32))
        v = jnp.dot(xblk, wb[:, 2 * D:3 * D], preferred_element_type=f32).astype(bf16)
        z_s[...] += jnp.sum(pk.reshape(BR // 8, 8, D), axis=0)
        pkb = pk.astype(bf16)
        for g in range(NG):
            kv_s[g] += lax.dot_general(pkb[:, g * 128:(g + 1) * 128], v[:, g * 128:(g + 1) * 128], TN,
                                       preferred_element_type=f32)
        return carry

    lax.fori_loop(0, S // BR, bkv_body, 0)

    rr = lax.broadcasted_iota(jnp.int32, (128, 128), 0) // DH
    cc_ = lax.broadcasted_iota(jnp.int32, (128, 128), 1) // DH
    same_head = rr == cc_
    for g in range(NG):
        kvm = jnp.where(same_head, kv_s[g], 0.0).astype(bf16)
        m_s[g * 128:(g + 1) * 128, :] = jnp.dot(
            kvm, wob[g * 128:(g + 1) * 128, :], preferred_element_type=f32).astype(bf16)
    ones_bd = jnp.where(same_head, 1.0, 0.0).astype(bf16)
    z_row = jnp.sum(z_s[...], axis=0, keepdims=True)

    def bq_body(i, carry):
        ro = pl.multiple_of(i * OR, OR)
        pq = _phi(jnp.dot(xb[pl.ds(ro, OR), :], wb[:, 0:D], preferred_element_type=f32))
        t = (pq * z_row).astype(bf16)
        den = jnp.concatenate(
            [jnp.dot(t[:, g * 128:(g + 1) * 128], ones_bd, preferred_element_type=f32) for g in range(NG)],
            axis=1) + 1e-6
        a = (pq / den).astype(bf16)
        y = jnp.dot(a, m_s[...], preferred_element_type=f32)
        ob_st[pl.ds(ro, OR), :] = y.astype(bf16)
        out_copy(ob_st, i, D, n_or + i).start()
        return carry

    lax.fori_loop(0, n_or, bq_body, 0)

    for i in range(n_or):
        out_copy(oa_st, i, 0, i).wait()
        out_copy(ob_st, i, D, n_or + i).wait()


@jax.jit
def pallas_concat_heads__mha_block__linear_attn_block__prompt_kernel(
    A_x: jax.Array,
    A_wqkv: jax.Array,
    A_wo: jax.Array,
    B_x: jax.Array,
    B_wqkv: jax.Array,
    B_wo: jax.Array,
):
    assert A_x.shape == (1, S, D) and B_x.shape == (1, S, D)
    any_spec = pl.BlockSpec(memory_space=pl.ANY)
    out = pl.pallas_call(
        _kernel,
        out_shape=jax.ShapeDtypeStruct((S, 2 * D), bf16),
        in_specs=[any_spec] * 6,
        out_specs=any_spec,
        scratch_shapes=[
            pltpu.VMEM((S, D), bf16),
            pltpu.VMEM((D, 3 * D), bf16),
            pltpu.VMEM((D, D), bf16),
            pltpu.VMEM((S, D), bf16),
            pltpu.VMEM((D, 3 * D), bf16),
            pltpu.VMEM((D, D), bf16),
            pltpu.VMEM((S, D), bf16),
            pltpu.VMEM((2, D, S), bf16),
            pltpu.VMEM((8, 128), bf16),
            pltpu.VMEM((D, S), bf16),
            pltpu.VMEM((S, TQ), f32),
            pltpu.VMEM((S, TQ), f32),
            pltpu.VMEM((NG, 128, 128), f32),
            pltpu.VMEM((8, D), f32),
            pltpu.VMEM((D, D), bf16),
            pltpu.VMEM((S, D), bf16),
            pltpu.VMEM((S, D), bf16),
            pltpu.SemaphoreType.DMA((11,)),
            pltpu.SemaphoreType.DMA((8,)),
        ],
        compiler_params=pltpu.CompilerParams(vmem_limit_bytes=120 * 1024 * 1024),
    )(A_x.reshape(S, D), A_wqkv, A_wo, B_x.reshape(S, D), B_wqkv, B_wo)
    return out.reshape(1, S, 2 * D)
```

```python
import math

import jax
import jax.numpy as jnp
from jax import lax
import jax.experimental.pallas as pl
import jax.experimental.pallas.tpu as pltpu

f32 = jnp.float32
bf16 = jnp.bfloat16

S = 2048
D = 1024
H = 32
DH = D // H
G = 128 // DH
NG = D // 128

TQ = 512
CK = 256
SUB = 32
SK = 1
UN = 8
NQ = S // TQ
NU = H * NQ
NC = S // CK
NS = CK // SUB
IPQ = H // UN
BC = 256

NT = (((1,), (1,)), ((), ()))
TN = (((0,), (0,)), ((), ()))

QSCALE = (DH ** -0.5) * math.log2(math.e)

OA_BLOCKS = [(0, 512), (512, 512), (1024, 512), (1536, 512)]
OB_BLOCKS = [(0, 512), (512, 512), (1024, 512), (1536, 256), (1792, 128), (1920, 128)]
X_CH = [(0, 128), (128, 128), (256, 256), (512, 512), (1024, 512), (1536, 512)]
W_CH = [(0, 128), (128, 128), (256, 256), (512, 512)]
N_IN = len(X_CH) + len(W_CH) + 2 + 4


def _phi(t):
    return jnp.where(t > 0, t + 1.0, jnp.exp(t)) + 1e-6


def _tr(w):
    return w.astype(f32).T.astype(bf16)


def _kernel(xa_hbm, wa_hbm, woa_hbm, xb_hbm, wb_hbm, wob_hbm, out_hbm,
            xa, wa, woa, xb, wb, wob,
            k_s, qt_s, vt_s, ot_s, sa, sb, at_s, m_s, wbt_s, oa_st, ob_st,
            in_sem, out_sem):
    in_copies = []

    def add_in(src, dst):
        cp = pltpu.make_async_copy(src, dst, in_sem.at[len(in_copies)])
        in_copies.append(cp)
        return cp

    c_xa = [add_in(xa_hbm.at[pl.ds(r, n), :], xa.at[pl.ds(r, n), :]) for r, n in X_CH]
    c_wk = [add_in(wa_hbm.at[:, pl.ds(D + c, n)], wa.at[:, pl.ds(D + c, n)]) for c, n in W_CH]
    c_wq = add_in(wa_hbm.at[:, pl.ds(0, D)], wa.at[:, pl.ds(0, D)])
    c_wv = add_in(wa_hbm.at[:, pl.ds(2 * D, D)], wa.at[:, pl.ds(2 * D, D)])
    c_woa = add_in(woa_hbm, woa)
    c_xb = add_in(xb_hbm, xb)
    c_wb = add_in(wb_hbm, wb)
    c_wob = add_in(wob_hbm, wob)
    assert len(in_copies) == N_IN

    for cp in (c_xa[0], c_wk[0], c_wk[1], c_xa[1], c_wk[2], c_xa[2], c_wk[3], *c_xa[3:], c_wq, c_wv,
               c_woa, c_xb, c_wb, c_wob):
        cp.start()

    def kproj(r0, r1, c0, c1):
        y = jnp.dot(xa[r0:r1, :], wa[:, D + c0:D + c1], preferred_element_type=f32)
        yb = y.astype(bf16)
        for g in range(c0 // 128, c1 // 128):
            k_s[g, r0:r1, :] = yb[:, g * 128 - c0:(g + 1) * 128 - c0]

    c_xa[0].wait(); c_wk[0].wait()
    kproj(0, 128, 0, 128)
    c_wk[1].wait()
    kproj(0, 128, 128, 256)
    c_xa[1].wait()
    kproj(128, 256, 0, 256)
    c_wk[2].wait()
    kproj(0, 256, 256, 512)
    c_xa[2].wait()
    kproj(256, 512, 0, 512)
    c_wk[3].wait()
    kproj(0, 512, 512, 1024)
    c_xa[3].wait()
    kproj(512, 1024, 0, 1024)
    c_xa[4].wait()
    kproj(1024, 1536, 0, 1024)
    c_xa[5].wait()
    c_wq.wait()
    c_wv.wait()
    kproj(1536, 2048, 0, 1024)

    WC = 512

    def qv(dst, wcol, co, scale):
        wt = _tr(wa[:, wcol + co:wcol + co + WC])
        for i in range(2):
            r = S // 2
            y = lax.dot_general(wt, xa[i * r:(i + 1) * r, :], NT, preferred_element_type=f32)
            if scale is not None:
                yb = (y * scale).astype(bf16)
                for q in range(r // TQ):
                    dst[i * (r // TQ) + q, co:co + WC, :] = yb[:, q * TQ:(q + 1) * TQ]
            else:
                dst[co:co + WC, i * r:(i + 1) * r] = y.astype(bf16)

    for co in range(0, D, WC):
        qv(qt_s, 0, co, QSCALE)
    for co in range(0, D, WC):
        qv(vt_s, 2 * D, co, None)

    bufs = (sa, sb)

    def offsets(it):
        if isinstance(it, int):
            return (it % IPQ) * (UN * DH), (it % IPQ) * (UN // G), it // IPQ
        lo = it & (IPQ - 1)
        fb = pl.multiple_of(lo * (UN * DH), UN * DH)
        return fb, lo * (UN // G), lax.shift_right_logical(it, IPQ.bit_length() - 1)

    def run(it, a_slots, c_slots, m_known, mp, extra=None):
        offs = {0: offsets(it)}
        if any(a is not None and a[0] >= UN for a in a_slots):
            offs[1] = offsets(it + 1)
        qms = {}
        prev_mh = None
        acc = None
        lhist = []
        for t, (a, cc) in enumerate(zip(a_slots, c_slots)):
            mh = None
            if a is not None:
                ua, c = a
                fb, gb, qi = offs[ua // UN]
                j_ = ua % UN
                if ua not in qms:
                    hh = j_ % G
                    qh = qt_s[qi, pl.ds(fb + j_ * DH, DH), :]
                    parts = []
                    if hh > 0:
                        parts.append(jnp.zeros((hh * DH, TQ), bf16))
                    parts.append(qh)
                    if hh < G - 1:
                        parts.append(jnp.zeros(((G - 1 - hh) * DH, TQ), bf16))
                    qms[ua] = jnp.concatenate(parts, axis=0)
                kg = k_s[gb + j_ // G, c * CK:(c + 1) * CK, :]
                s = jnp.dot(kg, qms[ua], preferred_element_type=f32)
                bufs[ua % 2][c * CK:(c + 1) * CK, :] = s
                mh = []
                for j in range(NS):
                    sm = jnp.max(s[j * SUB:(j + 1) * SUB].reshape(SUB // 8, 8, TQ), axis=0)
                    mp = sm if (c == 0 and j == 0) else jnp.maximum(mp, sm)
                    mh.append(mp)
                if c == NC - 1:
                    m_known[ua] = jnp.max(mp, axis=0, keepdims=True)
            elif extra is not None:
                extra(t)
            if cc is not None:
                uc, c = cc
                fb, gb, qi = offs[0]
                s_c = bufs[uc % 2]
                m_c = m_known[uc]
                if c == 0:
                    lhist = []
                ps_ = []
                for j in range(NS):
                    g = c * NS + j
                    r0 = c * CK + j * SUB
                    d0 = s_c[r0:r0 + 8, :] - m_c
                    if g >= 1:
                        d0 = jnp.minimum(d0, lhist[g - 1])
                    if prev_mh is not None:
                        d0 = jnp.minimum(d0, jnp.abs(prev_mh[j]))
                    d1 = s_c[r0 + 8:r0 + SUB, :] - m_c
                    p = jnp.exp2(jnp.concatenate([d0, d1], axis=0))
                    ps = jnp.sum(p.reshape(SUB // 8, 8, TQ), axis=0)
                    lhist.append(ps if g == 0 else lhist[-1] + ps)
                    ps_.append(p)
                pb = jnp.concatenate(ps_, axis=0).astype(bf16)
                vt = vt_s[pl.ds(fb + uc * DH, DH), c * CK:(c + 1) * CK]
                o = jnp.dot(vt, pb, preferred_element_type=f32)
                acc = o if c == 0 else acc + o
                if c == NC - 1:
                    l = jnp.sum(lhist[-1], axis=0, keepdims=True)
                    ot_s[qi, pl.ds(fb + uc * DH, DH), :] = (acc * (1.0 / l)).astype(bf16)
            prev_mh = mh
        return m_known, mp

    a0 = [(t // NC, t % NC) for t in range(NC + SK)]
    mk, mp0 = run(0, a0, [None] * len(a0), {}, None)

    n_slots = UN * NC
    a_sl = [((t + NC + SK) // NC, (t + NC + SK) % NC) for t in range(n_slots)]
    c_sl = [(t // NC, t % NC) for t in range(n_slots)]

    def att_body(i, carry):
        m0, mp, _ = carry
        mk_, mp = run(i, a_sl, c_sl, {0: m0}, mp)
        return mk_[UN], mp, i + 1

    n_it = NU // UN
    m_last, mp_last, it_last = lax.fori_loop(0, n_it - 1, att_body, (mk[0], mp0, jnp.int32(0)))

    out_copies = []

    def out_copy(st, r0, n, col):
        cp = pltpu.make_async_copy(
            st.at[pl.ds(r0, n), :], out_hbm.at[pl.ds(r0, n), pl.ds(col, D)], out_sem.at[len(out_copies)])
        out_copies.append(cp)
        cp.start()

    c_woa.wait()
    c_xb.wait()
    c_wb.wait()
    c_wob.wait()

    r0_, n_ = OA_BLOCKS[0]
    o_first = []
    npieces = 4
    pw = D // npieces
    first_free = n_slots - (NC + SK)

    def extra(t):
        k = t - first_free
        if k % 2 == 0 and k // 2 < npieces:
            if not o_first:
                o_first.append(_tr(ot_s[0]))
            c0 = (k // 2) * pw
            y = jnp.dot(o_first[0], woa[:, c0:c0 + pw], preferred_element_type=f32)
            oa_st[r0_:r0_ + n_, c0:c0 + pw] = y.astype(bf16)
        if k == 3:
            o_first.append(_tr(ot_s[1]))

    a_tail = [a if a[0] < UN else None for a in a_sl]
    run(it_last, a_tail, c_sl, {0: m_last}, mp_last, extra=extra)
    out_copy(oa_st, r0_, n_, 0)

    for bi, (r0, n) in enumerate(OA_BLOCKS[1:]):
        if bi == 0:
            y = jnp.dot(o_first[1], woa[...], preferred_element_type=f32)
        else:
            y = lax.dot_general(ot_s[bi + 1], woa[...], TN, preferred_element_type=f32)
        oa_st[r0:r0 + n, :] = y.astype(bf16)
        out_copy(oa_st, r0, n, 0)
        if bi < 2:
            for c0 in range(bi * D, (bi + 1) * D, 512):
                wbt_s[c0:c0 + 512, :] = _tr(wb[:, c0:c0 + 512])

    rr = lax.broadcasted_iota(jnp.int32, (128, 128), 0) // DH
    cc_ = lax.broadcasted_iota(jnp.int32, (128, 128), 1) // DH
    same_head = rr == cc_
    HB = BC // DH

    def b_body(r, carry):
        co = r * BC if isinstance(r, int) else pl.multiple_of(r * BC, BC)
        wkt = wbt_s[pl.ds(D + co, BC), :]
        pkt = _phi(lax.dot_general(wkt, xb[...], NT, preferred_element_type=f32))
        zp = pkt[:, 0:128]
        for j in range(1, S // 128):
            zp = zp + pkt[:, j * 128:(j + 1) * 128]
        z = jnp.sum(zp, axis=1, keepdims=True)
        t = jnp.dot(pkt.astype(bf16), xb[...], preferred_element_type=f32).astype(bf16)
        wqt = wbt_s[pl.ds(co, BC), :]
        nh = 4
        hw = S // nh
        for i in range(nh):
            pqt = _phi(lax.dot_general(wqt, xb[i * hw:(i + 1) * hw, :], NT, preferred_element_type=f32))
            den = jnp.sum((pqt * z).reshape(HB, DH, hw), axis=1, keepdims=True) + 1e-6
            at = pqt.reshape(HB, DH, hw) * (1.0 / den)
            at_s[r, i * hw:(i + 1) * hw, :] = at.reshape(BC, hw).T.astype(bf16)
            if i == nh - 2:
                kvs = []
                for g in range(BC // 128):
                    go = co + g * 128
                    kv = jnp.dot(t[g * 128:(g + 1) * 128, :], wb[:, pl.ds(2 * D + go, 128)],
                                 preferred_element_type=f32)
                    kvs.append(jnp.where(same_head, kv, 0.0).astype(bf16))
            if i == nh - 1:
                for g in range(BC // 128):
                    go = co + g * 128
                    m_s[pl.ds(go, 128), :] = jnp.dot(
                        kvs[g], wob[pl.ds(go, 128), :], preferred_element_type=f32).astype(bf16)
        return carry

    lax.fori_loop(0, D // BC, b_body, 0)

    for r0, n in OB_BLOCKS:
        a_blk = jnp.concatenate([at_s[r, r0:r0 + n, :] for r in range(D // BC)], axis=1)
        y = jnp.dot(a_blk, m_s[...], preferred_element_type=f32)
        ob_st[r0:r0 + n, :] = y.astype(bf16)
        out_copy(ob_st, r0, n, D)

    for cp in out_copies:
        cp.wait()


@jax.jit
def pallas_concat_heads__mha_block__linear_attn_block__prompt_kernel(
    A_x: jax.Array,
    A_wqkv: jax.Array,
    A_wo: jax.Array,
    B_x: jax.Array,
    B_wqkv: jax.Array,
    B_wo: jax.Array,
):
    assert A_x.shape == (1, S, D) and B_x.shape == (1, S, D)
    any_spec = pl.BlockSpec(memory_space=pl.ANY)
    out = pl.pallas_call(
        _kernel,
        out_shape=jax.ShapeDtypeStruct((S, 2 * D), bf16),
        in_specs=[any_spec] * 6,
        out_specs=any_spec,
        scratch_shapes=[
            pltpu.VMEM((S, D), bf16),
            pltpu.VMEM((D, 3 * D), bf16),
            pltpu.VMEM((D, D), bf16),
            pltpu.VMEM((S, D), bf16),
            pltpu.VMEM((D, 3 * D), bf16),
            pltpu.VMEM((D, D), bf16),
            pltpu.VMEM((NG, S, 128), bf16),
            pltpu.VMEM((NQ, D, TQ), bf16),
            pltpu.VMEM((D, S), bf16),
            pltpu.VMEM((NQ, D, TQ), bf16),
            pltpu.VMEM((S, TQ), f32),
            pltpu.VMEM((S, TQ), f32),
            pltpu.VMEM((D // BC, S, BC), bf16),
            pltpu.VMEM((D, D), bf16),
            pltpu.VMEM((2 * D, D), bf16),
            pltpu.VMEM((S, D), bf16),
            pltpu.VMEM((S, D), bf16),
            pltpu.SemaphoreType.DMA((N_IN,)),
            pltpu.SemaphoreType.DMA((len(OA_BLOCKS) + len(OB_BLOCKS),)),
        ],
        compiler_params=pltpu.CompilerParams(vmem_limit_bytes=120 * 1024 * 1024),
    )(A_x.reshape(S, D), A_wqkv, A_wo, B_x.reshape(S, D), B_wqkv, B_wo)
    return out.reshape(1, S, 2 * D)
```

```python
import math

import jax
import jax.numpy as jnp
from jax import lax
import jax.experimental.pallas as pl
import jax.experimental.pallas.tpu as pltpu

f32 = jnp.float32
bf16 = jnp.bfloat16

S = 2048
D = 1024
H = 32
DH = D // H
G = 128 // DH
NG = D // 128

TQ = 512
CK = 256
SUB = 16
SK = 1
UN = 12
UT = 8
NQ = S // TQ
NU = H * NQ
NC = S // CK
NS = CK // SUB

BC = 256
NB = D // BC
HB = BC // DH

NT = (((1,), (1,)), ((), ()))
TN = (((0,), (0,)), ((), ()))

QSCALE = (DH ** -0.5) * math.log2(math.e)

K_CH = [(0, 128), (128, 128), (256, 256), (512, 256), (768, 256)]
XH = 1024
OA_LAST = [(0, 256), (256, 128), (384, 64), (448, 64)]
N_SEM = len(K_CH) + 3


def _phi(t):
    return jnp.where(t > 0, t + 1.0, jnp.exp(t)) + 1e-6


def _tr(w):
    return w.astype(f32).T.astype(bf16)


def _kernel(xa_hbm, wa_hbm, woa_hbm, xb_hbm, wb_hbm, wob_hbm, out_hbm,
            xa, wa, woa, xb, wb, wob,
            k_s, qt_s, vt_s, ot_s, sa, sb, bacc, oa_st, ob_st, sem):
    groups = [[] for _ in range(N_SEM)]

    def copy(grp, src, dst):
        cp = pltpu.make_async_copy(src, dst, sem.at[grp])
        groups[grp].append(cp)
        cp.start()

    def wait(grp):
        for cp in groups[grp]:
            cp.wait()

    g_qv, g_b, g_out = len(K_CH), len(K_CH) + 1, len(K_CH) + 2
    for i, (k, n) in enumerate(K_CH):
        copy(i, xa_hbm.at[pl.ds(0, XH), pl.ds(k, n)], xa.at[pl.ds(0, XH), pl.ds(k, n)])
        copy(i, wa_hbm.at[pl.ds(k, n), pl.ds(D, D)], wa.at[pl.ds(k, n), pl.ds(D, D)])
    copy(len(K_CH) - 1, xa_hbm.at[pl.ds(XH, 512), :], xa.at[pl.ds(XH, 512), :])
    copy(g_qv, xa_hbm.at[pl.ds(XH + 512, 512), :], xa.at[pl.ds(XH + 512, 512), :])
    copy(g_qv, wa_hbm.at[:, pl.ds(0, D)], wa.at[:, pl.ds(0, D)])
    copy(g_qv, wa_hbm.at[:, pl.ds(2 * D, D)], wa.at[:, pl.ds(2 * D, D)])
    copy(g_b, xb_hbm, xb)
    for j in range(3 * NB):
        copy(g_b, wb_hbm.at[:, pl.ds(j * BC, BC)], wb.at[j])
    copy(g_b, wob_hbm, wob)
    copy(g_b, woa_hbm, woa)

    def out_copy(st, r0, n, col):
        copy(g_out, st.at[pl.ds(r0, n), :], out_hbm.at[pl.ds(r0, n), pl.ds(col, D)])

    def k_store(r0, r1, y):
        yb = y.astype(bf16)
        for g in range(NG):
            k_s[g, r0:r1, :] = yb[:, g * 128:(g + 1) * 128]

    def kproj(r0, r1):
        k_store(r0, r1, jnp.dot(xa[r0:r1, :], wa[:, D:2 * D], preferred_element_type=f32))

    for i, (k, n) in enumerate(K_CH):
        wait(i)
        y = jnp.dot(xa[0:XH, k:k + n], wa[k:k + n, D:2 * D], preferred_element_type=f32)
        if i > 0:
            y = y + jnp.concatenate([sa[0:XH, :], sa[XH:2 * XH, :]], axis=1)
        if i < len(K_CH) - 1:
            sa[0:XH, :] = y[:, 0:TQ]
            sa[XH:2 * XH, :] = y[:, TQ:2 * TQ]
        else:
            k_store(0, XH, y)
    kproj(XH, XH + 512)
    wait(g_qv)
    kproj(XH + 512, S)

    WC = 512
    XR = S // 2

    def proj_t(wcol, i):
        wt = _tr(wa[:, wcol:wcol + WC])
        return [lax.dot_general(wt, xa[i * XR:(i + 1) * XR, :], NT, preferred_element_type=f32)
                for i in range(S // XR)]

    for co in range(0, D, WC):
        for i, y in enumerate(proj_t(co, 0)):
            yb = (y * QSCALE).astype(bf16)
            for q in range(XR // TQ):
                qt_s[i * (XR // TQ) + q, co:co + WC, :] = yb[:, q * TQ:(q + 1) * TQ]
    for co in range(0, D, WC):
        for i, y in enumerate(proj_t(2 * D + co, 0)):
            vt_s[co:co + WC, i * XR:(i + 1) * XR] = y.astype(bf16)

    bufs = (sa, sb)

    def offsets(gidx):
        if isinstance(gidx, int):
            return (gidx % NG) * 128, gidx % NG, gidx // NG
        gb = gidx & (NG - 1)
        return pl.multiple_of(gb * 128, 128), gb, lax.shift_right_logical(gidx, NG.bit_length() - 1)

    def run(g0, a_slots, c_slots, m_known, mp, extra=None):
        offs = {}

        def off(u):
            if u // G not in offs:
                offs[u // G] = offsets(g0 + u // G)
            return offs[u // G]

        qms = {}
        prev_mh = None
        acc = None
        lhist = []
        for t, (a, cc) in enumerate(zip(a_slots, c_slots)):
            mh = None
            if a is not None:
                ua, c = a
                fb, gb, qi = off(ua)
                if ua not in qms:
                    hh = ua % G
                    qh = qt_s[qi, pl.ds(fb + hh * DH, DH), :]
                    parts = []
                    if hh > 0:
                        parts.append(jnp.zeros((hh * DH, TQ), bf16))
                    parts.append(qh)
                    if hh < G - 1:
                        parts.append(jnp.zeros(((G - 1 - hh) * DH, TQ), bf16))
                    qms[ua] = jnp.concatenate(parts, axis=0)
                kg = k_s[gb, c * CK:(c + 1) * CK, :]
                s = jnp.dot(kg, qms[ua], preferred_element_type=f32)
                bufs[ua % 2][c * CK:(c + 1) * CK, :] = s
                mh = []
                for j in range(NS):
                    sm = jnp.max(s[j * SUB:(j + 1) * SUB].reshape(SUB // 8, 8, TQ), axis=0)
                    mp = sm if (c == 0 and j == 0) else jnp.maximum(mp, sm)
                    mh.append(mp)
                if c == NC - 1:
                    m_known[ua] = jnp.max(mp, axis=0, keepdims=True)
            elif extra is not None:
                extra(t)
            if cc is not None:
                uc, c = cc
                fb, gb, qi = off(uc)
                ho = fb + (uc % G) * DH
                s_c = bufs[uc % 2]
                m_c = m_known[uc]
                if c == 0:
                    lhist = []
                ps_ = []
                for j in range(NS):
                    g = c * NS + j
                    r0 = c * CK + j * SUB
                    d0 = s_c[r0:r0 + 8, :] - m_c
                    if g >= 1:
                        d0 = jnp.minimum(d0, lhist[g - 1])
                    if prev_mh is not None and j % 2 == 1:
                        d0 = jnp.minimum(d0, jnp.abs(prev_mh[j]))
                    d1 = s_c[r0 + 8:r0 + SUB, :] - m_c
                    p = jnp.exp2(jnp.concatenate([d0, d1], axis=0))
                    ps = jnp.sum(p.reshape(SUB // 8, 8, TQ), axis=0)
                    lhist.append(ps if g == 0 else lhist[-1] + ps)
                    ps_.append(p)
                pb = jnp.concatenate(ps_, axis=0).astype(bf16)
                vt = vt_s[pl.ds(ho, DH), c * CK:(c + 1) * CK]
                o = jnp.dot(vt, pb, preferred_element_type=f32)
                acc = o if c == 0 else acc + o
                if c == NC - 1:
                    l = jnp.sum(lhist[-1], axis=0, keepdims=True)
                    ot_s[qi, pl.ds(ho, DH), :] = (acc * (1.0 / l)).astype(bf16)
            prev_mh = mh
        return m_known, mp

    def slots(n_units, lead):
        return [((t + lead) // NC, (t + lead) % NC) for t in range(n_units * NC)]

    a0 = slots(2, 0)[:NC + SK]
    mk, mp0 = run(0, a0, [None] * len(a0), {}, None)

    wait(g_b)
    same_head = (lax.broadcasted_iota(jnp.int32, (128, 128), 0) // DH
                 == lax.broadcasted_iota(jnp.int32, (128, 128), 1) // DH)

    def b_body(r, carry):
        pkt = _phi(jnp.dot(xb[...], wb[NB + r], preferred_element_type=f32)).T
        zp = pkt[:, 0:128]
        for j in range(1, S // 128):
            zp = zp + pkt[:, j * 128:(j + 1) * 128]
        z = jnp.sum(zp, axis=1, keepdims=True)
        t = jnp.dot(pkt.astype(bf16), xb[...], preferred_element_type=f32).astype(bf16)
        wqt = _tr(wb[r])
        nh = 4
        hw = S // nh
        a_rows = []
        for i in range(nh):
            pqt = _phi(lax.dot_general(wqt, xb[i * hw:(i + 1) * hw, :], NT, preferred_element_type=f32))
            den = jnp.sum((pqt * z).reshape(HB, DH, hw), axis=1, keepdims=True) + 1e-6
            at = pqt.reshape(HB, DH, hw) * (1.0 / den)
            a_rows.append(at.reshape(BC, hw).T.astype(bf16))
            if i == 1:
                kvs = []
                for g in range(BC // 128):
                    kv = jnp.dot(t[g * 128:(g + 1) * 128, :], wb[2 * NB + r, :, g * 128:(g + 1) * 128],
                                 preferred_element_type=f32)
                    kvs.append(jnp.where(same_head, kv, 0.0).astype(bf16))
            if i == 2:
                ms = []
                for g in range(BC // 128):
                    go = pl.multiple_of(r * BC + g * 128, 128)
                    ms.append(jnp.dot(kvs[g], wob[pl.ds(go, 128), :], preferred_element_type=f32).astype(bf16))
                m_r = jnp.concatenate(ms, axis=0)
        for i in range(nh):
            prev = jnp.where(r > 0, bacc[i * hw:(i + 1) * hw, :], 0.0)
            y = prev + jnp.dot(a_rows[i], m_r, preferred_element_type=f32)
            bacc[i * hw:(i + 1) * hw, :] = y
            ob_st[i * hw:(i + 1) * hw, :] = y.astype(bf16)
        return carry

    lax.fori_loop(0, NB, b_body, 0)
    out_copy(ob_st, 0, S, D)

    a_sl = slots(UN, NC + SK)
    c_sl = slots(UN, 0)

    def att_body(i, carry):
        m0, mp, _ = carry
        mk_, mp = run(i * (UN // G), a_sl, c_sl, {0: m0}, mp)
        return mk_[UN], mp, (i + 1) * (UN // G)

    n_it = (NU - UT) // UN
    assert n_it * UN + UT == NU and UN % G == 0 and UT % G == 0
    m_last, mp_last, g_last = lax.fori_loop(0, n_it, att_body, (mk[0], mp0, jnp.int32(0)))

    o_rows = []
    first_free = UT * NC - (NC + SK)

    def extra(t):
        k = t - first_free
        if k in (0, 4):
            if k == 0:
                o_rows.append(ot_s[0].T)
            c0 = (k // 4) * (D // 2)
            y = jnp.dot(o_rows[0], woa[:, c0:c0 + D // 2], preferred_element_type=f32)
            oa_st[0:TQ, c0:c0 + D // 2] = y.astype(bf16)
        if k == 3:
            o_rows.append(ot_s[1].T)

    a_tail = [a if a[0] < UT else None for a in slots(UT, NC + SK)]
    run(g_last, a_tail, slots(UT, 0), {0: m_last}, mp_last, extra=extra)
    out_copy(oa_st, 0, TQ, 0)

    oa_st[TQ:2 * TQ, :] = jnp.dot(o_rows[1], woa[...], preferred_element_type=f32).astype(bf16)
    out_copy(oa_st, TQ, TQ, 0)
    oa_st[2 * TQ:3 * TQ, :] = lax.dot_general(ot_s[2], woa[...], TN, preferred_element_type=f32).astype(bf16)
    out_copy(oa_st, 2 * TQ, TQ, 0)
    o_last = ot_s[3].T
    for p0, pn in OA_LAST:
        y = jnp.dot(o_last[p0:p0 + pn], woa[...], preferred_element_type=f32)
        oa_st[3 * TQ + p0:3 * TQ + p0 + pn, :] = y.astype(bf16)
        out_copy(oa_st, 3 * TQ + p0, pn, 0)

    wait(g_out)


@jax.jit
def pallas_concat_heads__mha_block__linear_attn_block__prompt_kernel(
    A_x: jax.Array,
    A_wqkv: jax.Array,
    A_wo: jax.Array,
    B_x: jax.Array,
    B_wqkv: jax.Array,
    B_wo: jax.Array,
):
    assert A_x.shape == (1, S, D) and B_x.shape == (1, S, D)
    any_spec = pl.BlockSpec(memory_space=pl.ANY)
    out = pl.pallas_call(
        _kernel,
        out_shape=jax.ShapeDtypeStruct((S, 2 * D), bf16),
        in_specs=[any_spec] * 6,
        out_specs=any_spec,
        scratch_shapes=[
            pltpu.VMEM((S, D), bf16),
            pltpu.VMEM((D, 3 * D), bf16),
            pltpu.VMEM((D, D), bf16),
            pltpu.VMEM((S, D), bf16),
            pltpu.VMEM((3 * NB, D, BC), bf16),
            pltpu.VMEM((D, D), bf16),
            pltpu.VMEM((NG, S, 128), bf16),
            pltpu.VMEM((NQ, D, TQ), bf16),
            pltpu.VMEM((D, S), bf16),
            pltpu.VMEM((NQ, D, TQ), bf16),
            pltpu.VMEM((S, TQ), f32),
            pltpu.VMEM((S, TQ), f32),
            pltpu.VMEM((S, D), f32),
            pltpu.VMEM((S, D), bf16),
            pltpu.VMEM((S, D), bf16),
            pltpu.SemaphoreType.DMA((N_SEM,)),
        ],
        compiler_params=pltpu.CompilerParams(vmem_limit_bytes=120 * 1024 * 1024),
    )(A_x.reshape(S, D), A_wqkv, A_wo, B_x.reshape(S, D), B_wqkv, B_wo)
    return out.reshape(1, S, 2 * D)
```

```python
import math

import jax
import jax.numpy as jnp
from jax import lax
import jax.experimental.pallas as pl
import jax.experimental.pallas.tpu as pltpu

f32 = jnp.float32
bf16 = jnp.bfloat16

S = 2048
D = 1024
H = 32
DH = D // H
G = 128 // DH
NG = D // 128

TQ = 512
CK = 256
SUB = 16
SK = 1
UN = 12
UT = 8
NQ = S // TQ
NU = H * NQ
NC = S // CK
NS = CK // SUB

NKV = 32
CX = 1
X0 = CX * CK
SEG = 92

BC = 256
NB = D // BC
HB = BC // DH

NT = (((1,), (1,)), ((), ()))
TN = (((0,), (0,)), ((), ()))

QSCALE = (DH ** -0.5) * math.log2(math.e)

K_CH = [(0, 128), (128, 128), (256, 256), (512, 256), (768, 256)]
XH = 1024
OA_LAST = [(0, 256), (256, 128), (384, 64), (448, 64)]
N_SEM = len(K_CH) + 3


def _phi(t):
    return jnp.where(t > 0, t + 1.0, jnp.exp(t)) + 1e-6


def _tr(w):
    return w.astype(f32).T.astype(bf16)


def _kernel(xa_hbm, wa_hbm, woa_hbm, xb_hbm, wb_hbm, wob_hbm, out_hbm,
            xa, wa, woa, xb, wb, wob,
            k_s, qt_s, vt_s, ot_s, sa, sb, bacc, oa_st, ob_st, sx_s, one_s, qf_s, kf_s, sem):
    groups = [[] for _ in range(N_SEM)]

    def copy(grp, src, dst):
        cp = pltpu.make_async_copy(src, dst, sem.at[grp])
        groups[grp].append(cp)
        cp.start()

    def wait(grp):
        for cp in groups[grp]:
            cp.wait()

    g_qv, g_b, g_out = len(K_CH), len(K_CH) + 1, len(K_CH) + 2
    for i, (k, n) in enumerate(K_CH):
        copy(i, xa_hbm.at[pl.ds(0, XH), pl.ds(k, n)], xa.at[pl.ds(0, XH), pl.ds(k, n)])
        copy(i, wa_hbm.at[pl.ds(k, n), pl.ds(D, D)], wa.at[pl.ds(k, n), pl.ds(D, D)])
    copy(len(K_CH) - 1, xa_hbm.at[pl.ds(XH, 512), :], xa.at[pl.ds(XH, 512), :])
    copy(g_qv, xa_hbm.at[pl.ds(XH + 512, 512), :], xa.at[pl.ds(XH + 512, 512), :])
    copy(g_qv, wa_hbm.at[:, pl.ds(0, D)], wa.at[:, pl.ds(0, D)])
    copy(g_qv, wa_hbm.at[:, pl.ds(2 * D, D)], wa.at[:, pl.ds(2 * D, D)])
    copy(g_b, xb_hbm, xb)
    for j in range(3 * NB):
        copy(g_b, wb_hbm.at[:, pl.ds(j * BC, BC)], wb.at[j])
    copy(g_b, wob_hbm, wob)
    copy(g_b, woa_hbm, woa)

    def out_copy(st, r0, n, col):
        copy(g_out, st.at[pl.ds(r0, n), :], out_hbm.at[pl.ds(r0, n), pl.ds(col, D)])

    def k_store(r0, r1, y):
        yb = y.astype(bf16)
        for g in range(NG):
            k_s[g, r0:r1, :] = yb[:, g * 128:(g + 1) * 128]
            if r0 <= X0 < r1:
                kf_s[g] = y[X0 - r0:X0 - r0 + NKV, g * 128:(g + 1) * 128]

    def kproj(r0, r1):
        k_store(r0, r1, jnp.dot(xa[r0:r1, :], wa[:, D:2 * D], preferred_element_type=f32))

    bacc[...] = jnp.zeros_like(bacc)
    for i, (k, n) in enumerate(K_CH):
        wait(i)
        y = jnp.dot(xa[0:XH, k:k + n], wa[k:k + n, D:2 * D], preferred_element_type=f32)
        if i > 0:
            y = y + jnp.concatenate([sa[0:XH, :], sa[XH:2 * XH, :]], axis=1)
        if i < len(K_CH) - 1:
            sa[0:XH, :] = y[:, 0:TQ]
            sa[XH:2 * XH, :] = y[:, TQ:2 * TQ]
        else:
            k_store(0, XH, y)
    kproj(XH, XH + 512)
    wait(g_qv)
    kproj(XH + 512, S)

    WC = 512
    XR = S // 2

    def proj_t(wcol):
        wt = _tr(wa[:, wcol:wcol + WC])
        return [lax.dot_general(wt, xa[i * XR:(i + 1) * XR, :], NT, preferred_element_type=f32)
                for i in range(S // XR)]

    for co in range(0, D, WC):
        for i, y in enumerate(proj_t(co)):
            ys = y * QSCALE
            yb = ys.astype(bf16)
            for q in range(XR // TQ):
                qf_s[i * (XR // TQ) + q, co:co + WC, :] = ys[:, q * TQ:(q + 1) * TQ]
                qt_s[i * (XR // TQ) + q, co:co + WC, :] = yb[:, q * TQ:(q + 1) * TQ]
    for co in range(0, D, WC):
        for i, y in enumerate(proj_t(2 * D + co)):
            vt_s[co:co + WC, i * XR:(i + 1) * XR] = y.astype(bf16)

    bufs = (sa, sb)

    def offsets(gidx):
        if isinstance(gidx, int):
            return (gidx % NG) * 128, gidx % NG, gidx // NG
        gb = gidx & (NG - 1)
        return pl.multiple_of(gb * 128, 128), gb, lax.shift_right_logical(gidx, NG.bit_length() - 1)

    def run(g0, a_slots, c_slots, m_known, mp, extra=None, use_sx=True):
        offs = {}

        def off(u):
            if u // G not in offs:
                offs[u // G] = offsets(g0 + u // G)
            return offs[u // G]

        qms = {}
        prev_mh = None
        acc = None
        lhist = []
        for t, (a, cc) in enumerate(zip(a_slots, c_slots)):
            mh = None
            if a is not None:
                ua, c = a
                fb, gb, qi = off(ua)
                if ua not in qms:
                    hh = ua % G
                    qh = qt_s[qi, pl.ds(fb + hh * DH, DH), :]
                    parts = []
                    if hh > 0:
                        parts.append(jnp.zeros((hh * DH, TQ), bf16))
                    parts.append(qh)
                    if hh < G - 1:
                        parts.append(jnp.zeros(((G - 1 - hh) * DH, TQ), bf16))
                    qms[ua] = jnp.concatenate(parts, axis=0)
                if use_sx and c == CX:
                    kg = k_s[gb, X0 + NKV:(c + 1) * CK, :]
                    s = jnp.concatenate([sx_s[qi * H + gb * G + ua % G],
                                         jnp.dot(kg, qms[ua], preferred_element_type=f32)], axis=0)
                else:
                    kg = k_s[gb, c * CK:(c + 1) * CK, :]
                    s = jnp.dot(kg, qms[ua], preferred_element_type=f32)
                bufs[ua % 2][c * CK:(c + 1) * CK, :] = s
                mh = []
                for j in range(NS):
                    sm = jnp.max(s[j * SUB:(j + 1) * SUB].reshape(SUB // 8, 8, TQ), axis=0)
                    mp = sm if (c == 0 and j == 0) else jnp.maximum(mp, sm)
                    mh.append(mp)
                if c == NC - 1:
                    m_known[ua] = jnp.max(mp, axis=0, keepdims=True)
            elif extra is not None:
                extra(t)
            if cc is not None:
                uc, c = cc
                fb, gb, qi = off(uc)
                ho = fb + (uc % G) * DH
                s_c = bufs[uc % 2]
                m_c = m_known[uc]
                if c == 0:
                    lhist = []
                ps_ = []
                for j in range(NS):
                    g = c * NS + j
                    r0 = c * CK + j * SUB
                    d0 = s_c[r0:r0 + 8, :] - m_c
                    if g >= 1:
                        d0 = jnp.minimum(d0, lhist[g - 1])
                    if prev_mh is not None and j % 2 == 1:
                        d0 = jnp.minimum(d0, jnp.abs(prev_mh[j]))
                    d1 = s_c[r0 + 8:r0 + SUB, :] - m_c
                    p = jnp.exp2(jnp.concatenate([d0, d1], axis=0))
                    ps = jnp.sum(p.reshape(SUB // 8, 8, TQ), axis=0)
                    lhist.append(ps if g == 0 else lhist[-1] + ps)
                    ps_.append(p)
                pb = jnp.concatenate(ps_, axis=0).astype(bf16)
                vt = vt_s[pl.ds(ho, DH), c * CK:(c + 1) * CK]
                o = jnp.dot(vt, pb, preferred_element_type=f32)
                acc = o if c == 0 else acc + o
                if c == NC - 1:
                    l = jnp.sum(lhist[-1], axis=0, keepdims=True)
                    ot_s[qi, pl.ds(ho, DH), :] = (acc * (1.0 / l)).astype(bf16)
            prev_mh = mh
        return m_known, mp

    def slots(n_units, lead):
        return [((t + lead) // NC, (t + lead) % NC) for t in range(n_units * NC)]

    a0 = slots(2, 0)[:NC + SK]
    mk, mp0 = run(0, a0, [None] * len(a0), {}, None, use_sx=False)

    one_s[...] = jnp.ones_like(one_s)
    wait(g_b)
    same_head = (lax.broadcasted_iota(jnp.int32, (128, 128), 0) // DH
                 == lax.broadcasted_iota(jnp.int32, (128, 128), 1) // DH)

    def b_body(r, carry):
        co = pl.multiple_of(r * BC, BC)
        always = one_s[...] > 0.0
        always2 = one_s[...] > 0.5
        pieces = [(hh, qi, q0) for hh in range(HB) for qi in range(NQ) for q0 in range(0, TQ, 128)]
        kbs = {}
        ng = NKV // 8

        def vpu_scores(todo, link, slow):
            fin = None
            for hh, qi, q0 in todo:
                if hh not in kbs:
                    k32 = kf_s[r * (BC // 128) + hh // G]
                    l0 = (hh % G) * DH
                    kbs[hh] = [jnp.broadcast_to(k32[:, l0 + d:l0 + d + 1], (NKV, 128)) for d in range(DH)]
                q32 = qf_s[qi, pl.ds(co + hh * DH, DH), q0:q0 + 128]
                acc = None
                for d in range(DH):
                    qd = jnp.broadcast_to(q32[d:d + 1, :], (8, 128))
                    if link is not None:
                        qd = jnp.where(always, qd, link)
                    if fin is not None and 1 <= d < ng:
                        gf = (DH - 1 + d) % ng
                        qd = jnp.where(always, qd, fin[gf * 8:(gf + 1) * 8])
                    if slow and link is not None:
                        qd = jnp.where(always2, qd, link)
                    t_ = kbs[hh][d] * jnp.concatenate([qd] * ng, axis=0)
                    acc = t_ if acc is None else acc + t_
                    link = acc[(d % ng) * 8:(d % ng + 1) * 8]
                sx_s[qi * H + r * HB + hh, :, q0:q0 + 128] = acc
                fin = acc
            return fin

        link1 = vpu_scores(pieces[:SEG], None, False)
        pkt = _phi(jnp.dot(xb[...], wb[NB + r], preferred_element_type=f32)).T
        zp = pkt[:, 0:128]
        for j in range(1, S // 128):
            zp = zp + pkt[:, j * 128:(j + 1) * 128]
        z = jnp.sum(zp, axis=1, keepdims=True)
        t = jnp.dot(pkt.astype(bf16), xb[...], preferred_element_type=f32).astype(bf16)
        w32 = wb[r].astype(f32)
        w00 = jnp.where(jnp.concatenate([always] * ng, axis=0), w32[0:NKV, 0:128], link1)
        w32 = jnp.concatenate([jnp.concatenate([w00, w32[0:NKV, 128:]], axis=1), w32[NKV:]], axis=0)
        wqt = w32.T.astype(bf16)
        nh = 4
        hw = S // nh
        a_rows = []
        for i in range(nh):
            pqt = _phi(lax.dot_general(wqt, xb[i * hw:(i + 1) * hw, :], NT, preferred_element_type=f32))
            den = jnp.sum((pqt * z).reshape(HB, DH, hw), axis=1, keepdims=True) + 1e-6
            at = pqt.reshape(HB, DH, hw) * (1.0 / den)
            a_rows.append(at.reshape(BC, hw).T.astype(bf16))
            if i == nh - 1:
                link2 = at.reshape(BC, hw)[BC - 8:BC, hw - 128:hw]
            if i == 1:
                kvs = []
                for g in range(BC // 128):
                    kv = jnp.dot(t[g * 128:(g + 1) * 128, :], wb[2 * NB + r, :, g * 128:(g + 1) * 128],
                                 preferred_element_type=f32)
                    kvs.append(jnp.where(same_head, kv, 0.0).astype(bf16))
            if i == 2:
                ms = []
                for g in range(BC // 128):
                    go = pl.multiple_of(r * BC + g * 128, 128)
                    ms.append(jnp.dot(kvs[g], wob[pl.ds(go, 128), :], preferred_element_type=f32).astype(bf16))
                m_r = jnp.concatenate(ms, axis=0)
        vpu_scores(pieces[SEG:], link2, True)
        for i in range(nh):
            y = bacc[i * hw:(i + 1) * hw, :] + jnp.dot(a_rows[i], m_r, preferred_element_type=f32)
            bacc[i * hw:(i + 1) * hw, :] = y
            ob_st[i * hw:(i + 1) * hw, :] = y.astype(bf16)
        return carry

    lax.fori_loop(0, NB, b_body, 0)
    out_copy(ob_st, 0, S, D)

    a_sl = slots(UN, NC + SK)
    c_sl = slots(UN, 0)

    def att_body(i, carry):
        m0, mp, _ = carry
        mk_, mp = run(i * (UN // G), a_sl, c_sl, {0: m0}, mp)
        return mk_[UN], mp, (i + 1) * (UN // G)

    n_it = (NU - UT) // UN
    assert n_it * UN + UT == NU and UN % G == 0 and UT % G == 0
    m_last, mp_last, g_last = lax.fori_loop(0, n_it, att_body, (mk[0], mp0, jnp.int32(0)))

    o_rows = []
    first_free = UT * NC - (NC + SK)

    def extra(t):
        k = t - first_free
        if k in (0, 4):
            if k == 0:
                o_rows.append(ot_s[0].T)
            c0 = (k // 4) * (D // 2)
            y = jnp.dot(o_rows[0], woa[:, c0:c0 + D // 2], preferred_element_type=f32)
            oa_st[0:TQ, c0:c0 + D // 2] = y.astype(bf16)
        if k == 3:
            o_rows.append(ot_s[1].T)

    a_tail = [a if a[0] < UT else None for a in slots(UT, NC + SK)]
    run(g_last, a_tail, slots(UT, 0), {0: m_last}, mp_last, extra=extra)
    out_copy(oa_st, 0, TQ, 0)

    oa_st[TQ:2 * TQ, :] = jnp.dot(o_rows[1], woa[...], preferred_element_type=f32).astype(bf16)
    out_copy(oa_st, TQ, TQ, 0)
    oa_st[2 * TQ:3 * TQ, :] = lax.dot_general(ot_s[2], woa[...], TN, preferred_element_type=f32).astype(bf16)
    out_copy(oa_st, 2 * TQ, TQ, 0)
    o_last = ot_s[3].T
    for p0, pn in OA_LAST:
        y = jnp.dot(o_last[p0:p0 + pn], woa[...], preferred_element_type=f32)
        oa_st[3 * TQ + p0:3 * TQ + p0 + pn, :] = y.astype(bf16)
        out_copy(oa_st, 3 * TQ + p0, pn, 0)

    wait(g_out)


@jax.jit
def pallas_concat_heads__mha_block__linear_attn_block__prompt_kernel(
    A_x: jax.Array,
    A_wqkv: jax.Array,
    A_wo: jax.Array,
    B_x: jax.Array,
    B_wqkv: jax.Array,
    B_wo: jax.Array,
):
    assert A_x.shape == (1, S, D) and B_x.shape == (1, S, D)
    any_spec = pl.BlockSpec(memory_space=pl.ANY)
    out = pl.pallas_call(
        _kernel,
        out_shape=jax.ShapeDtypeStruct((S, 2 * D), bf16),
        in_specs=[any_spec] * 6,
        out_specs=any_spec,
        scratch_shapes=[
            pltpu.VMEM((S, D), bf16),
            pltpu.VMEM((D, 3 * D), bf16),
            pltpu.VMEM((D, D), bf16),
            pltpu.VMEM((S, D), bf16),
            pltpu.VMEM((3 * NB, D, BC), bf16),
            pltpu.VMEM((D, D), bf16),
            pltpu.VMEM((NG, S, 128), bf16),
            pltpu.VMEM((NQ, D, TQ), bf16),
            pltpu.VMEM((D, S), bf16),
            pltpu.VMEM((NQ, D, TQ), bf16),
            pltpu.VMEM((S, TQ), f32),
            pltpu.VMEM((S, TQ), f32),
            pltpu.VMEM((S, D), f32),
            pltpu.VMEM((S, D), bf16),
            pltpu.VMEM((S, D), bf16),
            pltpu.VMEM((NU, NKV, TQ), f32),
            pltpu.VMEM((8, 128), f32),
            pltpu.VMEM((NQ, D, TQ), f32),
            pltpu.VMEM((NG, NKV, 128), f32),
            pltpu.SemaphoreType.DMA((N_SEM,)),
        ],
        compiler_params=pltpu.CompilerParams(vmem_limit_bytes=120 * 1024 * 1024),
    )(A_x.reshape(S, D), A_wqkv, A_wo, B_x.reshape(S, D), B_wqkv, B_wo)
    return out.reshape(1, S, 2 * D)
```

```python
import math

import jax
import jax.numpy as jnp
from jax import lax
import jax.experimental.pallas as pl
import jax.experimental.pallas.tpu as pltpu

f32 = jnp.float32
bf16 = jnp.bfloat16

S = 2048
D = 1024
H = 32
DH = D // H
G = 128 // DH
NG = D // 128

TQ = 512
CK = 256
SUB = 16
SK = 1
UN = 12
UT = 8
NQ = S // TQ
NU = H * NQ
NC = S // CK
NS = CK // SUB

NKV = 32
CX, CX2 = 1, 3
X0, X2 = CX * CK, CX2 * CK
SEG = 100


def _second(gidx, hh):
    return hh >= 2 or (hh == 1 and gidx % (UN // G) < 2)


BC = 256
NB = D // BC
HB = BC // DH

NT = (((1,), (1,)), ((), ()))
TN = (((0,), (0,)), ((), ()))

QSCALE = (DH ** -0.5) * math.log2(math.e)

K_CH = [(0, 128), (128, 128), (256, 256), (512, 256), (768, 256)]
XH = 1024
OA_LAST = [(0, 256), (256, 128), (384, 64), (448, 64)]
N_SEM = len(K_CH) + 3


def _phi(t):
    return jnp.where(t > 0, t + 1.0, jnp.exp(t)) + 1e-6


def _kernel(xa_hbm, wa_hbm, woa_hbm, xb_hbm, wb_hbm, wob_hbm, out_hbm,
            xa, wa, woa, xb, wb, wob,
            k_s, qt_s, vt_s, ot_s, sa, sb, bacc, oa_st, ob_st, sx_s, one_s, qf_s, kf_s, sx2_s, kf2_s, sem):
    groups = [[] for _ in range(N_SEM)]

    def copy(grp, src, dst):
        cp = pltpu.make_async_copy(src, dst, sem.at[grp])
        groups[grp].append(cp)
        cp.start()

    def wait(grp):
        for cp in groups[grp]:
            cp.wait()

    g_qv, g_b, g_out = len(K_CH), len(K_CH) + 1, len(K_CH) + 2
    for i, (k, n) in enumerate(K_CH):
        copy(i, xa_hbm.at[pl.ds(0, XH), pl.ds(k, n)], xa.at[pl.ds(0, XH), pl.ds(k, n)])
        copy(i, wa_hbm.at[pl.ds(k, n), pl.ds(D, D)], wa.at[pl.ds(k, n), pl.ds(D, D)])
    copy(len(K_CH) - 1, xa_hbm.at[pl.ds(XH, 512), :], xa.at[pl.ds(XH, 512), :])
    copy(g_qv, xa_hbm.at[pl.ds(XH + 512, 512), :], xa.at[pl.ds(XH + 512, 512), :])
    copy(g_qv, wa_hbm.at[:, pl.ds(0, D)], wa.at[:, pl.ds(0, D)])
    copy(g_qv, wa_hbm.at[:, pl.ds(2 * D, D)], wa.at[:, pl.ds(2 * D, D)])
    copy(g_b, xb_hbm, xb)
    for j in range(3 * NB):
        copy(g_b, wb_hbm.at[:, pl.ds(j * BC, BC)], wb.at[j])
    copy(g_b, wob_hbm, wob)
    copy(g_b, woa_hbm, woa)

    def out_copy(st, r0, n, col):
        copy(g_out, st.at[pl.ds(r0, n), :], out_hbm.at[pl.ds(r0, n), pl.ds(col, D)])

    def k_store(r0, r1, y):
        yb = y.astype(bf16)
        for g in range(NG):
            k_s[g, r0:r1, :] = yb[:, g * 128:(g + 1) * 128]
            if r0 <= X0 < r1:
                kf_s[g] = y[X0 - r0:X0 - r0 + NKV, g * 128:(g + 1) * 128]
            if r0 <= X2 < r1:
                kf2_s[g] = y[X2 - r0:X2 - r0 + NKV, g * 128:(g + 1) * 128]

    def kproj(r0, r1):
        k_store(r0, r1, jnp.dot(xa[r0:r1, :], wa[:, D:2 * D], preferred_element_type=f32))

    def zero_body(i, carry):
        bacc[pl.ds(pl.multiple_of(i * 128, 128), 128), :] = jnp.zeros((128, D), f32)
        return carry

    lax.fori_loop(0, S // 128, zero_body, 0)
    one_s[...] = jnp.ones_like(one_s)
    for i, (k, n) in enumerate(K_CH):
        wait(i)
        y = jnp.dot(xa[0:XH, k:k + n], wa[k:k + n, D:2 * D], preferred_element_type=f32)
        if i > 0:
            y = y + jnp.concatenate([sa[0:XH, :], sa[XH:2 * XH, :]], axis=1)
        if i < len(K_CH) - 1:
            sa[0:XH, :] = y[:, 0:TQ]
            sa[XH:2 * XH, :] = y[:, TQ:2 * TQ]
        else:
            k_store(0, XH, y)
    kproj(XH, XH + 512)
    wait(g_qv)
    kproj(XH + 512, S)

    ng = NKV // 8

    def vpu_scores(kf, sx, kbs, todo, link, slow):
        always = one_s[...] > 0.0
        always2 = one_s[...] > 0.5
        fin = None
        for grp, hh, row0, qi, q0, dst in todo:
            if hh not in kbs:
                k32 = kf[grp]
                l0 = (hh % G) * DH
                kbs[hh] = [jnp.broadcast_to(k32[:, l0 + d:l0 + d + 1], (NKV, 128)) for d in range(DH)]
            q32 = qf_s[qi, pl.ds(row0, DH), q0:q0 + 128]
            acc = None
            for d in range(DH):
                qd = jnp.broadcast_to(q32[d:d + 1, :], (8, 128))
                if link is not None:
                    qd = jnp.where(always, qd, link)
                if fin is not None and 1 <= d < ng:
                    gf = (DH - 1 + d) % ng
                    qd = jnp.where(always, qd, fin[gf * 8:(gf + 1) * 8])
                if slow and link is not None:
                    qd = jnp.where(always2, qd, link)
                t_ = kbs[hh][d] * jnp.concatenate([qd] * ng, axis=0)
                acc = t_ if acc is None else acc + t_
                link = acc[(d % ng) * 8:(d % ng + 1) * 8]
            sx[dst, :, q0:q0 + 128] = acc
            fin = acc
        return fin

    WC = 512
    XR = S // 2

    def proj_t(wcol):
        wt = wa[:, wcol:wcol + WC].T
        return [lax.dot_general(wt, xa[i * XR:(i + 1) * XR, :], NT, preferred_element_type=f32)
                for i in range(S // XR)]

    for co in range(0, D, WC):
        for i, y in enumerate(proj_t(co)):
            ys = y * QSCALE
            yb = ys.astype(bf16)
            for q in range(XR // TQ):
                qf_s[i * (XR // TQ) + q, co:co + WC, :] = ys[:, q * TQ:(q + 1) * TQ]
                qt_s[i * (XR // TQ) + q, co:co + WC, :] = yb[:, q * TQ:(q + 1) * TQ]
    vpu_scores(kf2_s, sx2_s, {},
               [(g, g * G + hh, (g * G + hh) * DH, qi, q0, (qi * NG + g) * 3 + hh - 1)
                for g0 in range(0, NG, WC // 128) for qi in range(NQ) for g in range(g0, g0 + WC // 128)
                for hh in range(1, G) if _second(qi * NG + g, hh) for q0 in range(0, TQ, 128)],
               None, True)
    for co in range(0, D, WC):
        for i, y in enumerate(proj_t(2 * D + co)):
            vt_s[co:co + WC, i * XR:(i + 1) * XR] = y.astype(bf16)

    bufs = (sa, sb)

    def offsets(gidx):
        if isinstance(gidx, int):
            return (gidx % NG) * 128, gidx % NG, gidx // NG
        gb = gidx & (NG - 1)
        return pl.multiple_of(gb * 128, 128), gb, lax.shift_right_logical(gidx, NG.bit_length() - 1)

    def run(g0, a_slots, c_slots, m_known, mp, extra=None, use_sx=True):
        offs = {}

        def off(u):
            if u // G not in offs:
                offs[u // G] = offsets(g0 + u // G)
            return offs[u // G]

        qms = {}
        prev_mh = None
        acc = None
        lhist = []
        for t, (a, cc) in enumerate(zip(a_slots, c_slots)):
            mh = None
            if a is not None:
                ua, c = a
                fb, gb, qi = off(ua)
                if ua not in qms:
                    hh = ua % G
                    qh = qt_s[qi, pl.ds(fb + hh * DH, DH), :]
                    parts = []
                    if hh > 0:
                        parts.append(jnp.zeros((hh * DH, TQ), bf16))
                    parts.append(qh)
                    if hh < G - 1:
                        parts.append(jnp.zeros(((G - 1 - hh) * DH, TQ), bf16))
                    qms[ua] = jnp.concatenate(parts, axis=0)
                if use_sx and c == CX:
                    kg = k_s[gb, X0 + NKV:(c + 1) * CK, :]
                    s = jnp.concatenate([sx_s[qi * H + gb * G + ua % G],
                                         jnp.dot(kg, qms[ua], preferred_element_type=f32)], axis=0)
                elif use_sx and c == CX2 and _second(ua // G, ua % G):
                    kg = k_s[gb, X2 + NKV:(c + 1) * CK, :]
                    s = jnp.concatenate([sx2_s[(qi * NG + gb) * 3 + ua % G - 1],
                                         jnp.dot(kg, qms[ua], preferred_element_type=f32)], axis=0)
                else:
                    kg = k_s[gb, c * CK:(c + 1) * CK, :]
                    s = jnp.dot(kg, qms[ua], preferred_element_type=f32)
                bufs[ua % 2][c * CK:(c + 1) * CK, :] = s
                mh = []
                for j in range(NS):
                    sm = jnp.max(s[j * SUB:(j + 1) * SUB].reshape(SUB // 8, 8, TQ), axis=0)
                    mp = sm if (c == 0 and j == 0) else jnp.maximum(mp, sm)
                    mh.append(mp)
                if c == NC - 1:
                    m_known[ua] = jnp.max(mp, axis=0, keepdims=True)
            elif extra is not None:
                extra(t)
            if cc is not None:
                uc, c = cc
                fb, gb, qi = off(uc)
                ho = fb + (uc % G) * DH
                s_c = bufs[uc % 2]
                m_c = m_known[uc]
                if c == 0:
                    lhist = []
                ps_ = []
                for j in range(NS):
                    g = c * NS + j
                    r0 = c * CK + j * SUB
                    d0 = s_c[r0:r0 + 8, :] - m_c
                    if g >= 1:
                        d0 = jnp.minimum(d0, lhist[g - 1])
                    if prev_mh is not None and j % 2 == 1:
                        d0 = jnp.minimum(d0, jnp.abs(prev_mh[j]))
                    d1 = s_c[r0 + 8:r0 + SUB, :] - m_c
                    p = jnp.exp2(jnp.concatenate([d0, d1], axis=0))
                    ps = jnp.sum(p.reshape(SUB // 8, 8, TQ), axis=0)
                    lhist.append(ps if g == 0 else lhist[-1] + ps)
                    ps_.append(p)
                pb = jnp.concatenate(ps_, axis=0).astype(bf16)
                vt = vt_s[pl.ds(ho, DH), c * CK:(c + 1) * CK]
                o = jnp.dot(vt, pb, preferred_element_type=f32)
                acc = o if c == 0 else acc + o
                if c == NC - 1:
                    l = jnp.sum(lhist[-1], axis=0, keepdims=True)
                    ot_s[qi, pl.ds(ho, DH), :] = (acc * (1.0 / l)).astype(bf16)
            prev_mh = mh
        return m_known, mp

    def slots(n_units, lead):
        return [((t + lead) // NC, (t + lead) % NC) for t in range(n_units * NC)]

    a0 = slots(2, 0)[:NC + SK]
    mk, mp0 = run(0, a0, [None] * len(a0), {}, None, use_sx=False)

    wait(g_b)
    same_head = (lax.broadcasted_iota(jnp.int32, (128, 128), 0) // DH
                 == lax.broadcasted_iota(jnp.int32, (128, 128), 1) // DH)

    def b_body(r, carry):
        co = pl.multiple_of(r * BC, BC)
        always = one_s[...] > 0.0
        pieces = [(r * (BC // 128) + hh // G, hh, co + hh * DH, qi, q0, qi * H + r * HB + hh)
                  for hh in range(HB) for qi in range(NQ) for q0 in range(0, TQ, 128)]
        kbs = {}
        link1 = vpu_scores(kf_s, sx_s, kbs, pieces[:SEG], None, False)
        pk = _phi(jnp.dot(xb[...], wb[NB + r], preferred_element_type=f32))
        z8 = jnp.sum(pk.reshape(S // 8, 8, BC), axis=0)
        z = jnp.sum(z8.T, axis=1, keepdims=True)
        t = jnp.dot(pk.astype(bf16).T, xb[...], preferred_element_type=f32).astype(bf16)
        w32 = wb[r].astype(f32)
        w00 = jnp.where(jnp.concatenate([always] * ng, axis=0), w32[0:NKV, 0:128], link1)
        w32 = jnp.concatenate([jnp.concatenate([w00, w32[0:NKV, 128:]], axis=1), w32[NKV:]], axis=0)
        wqt = w32.T.astype(bf16)
        nh = 4
        hw = S // nh
        a_rows = []
        for i in range(nh):
            pqt = _phi(lax.dot_general(wqt, xb[i * hw:(i + 1) * hw, :], NT, preferred_element_type=f32))
            den = jnp.sum((pqt * z).reshape(HB, DH, hw), axis=1, keepdims=True) + 1e-6
            at = pqt.reshape(HB, DH, hw) * (1.0 / den)
            a_rows.append(at.reshape(BC, hw).T.astype(bf16))
            if i == nh - 1:
                link2 = at.reshape(BC, hw)[BC - 8:BC, hw - 128:hw]
            if i == 1:
                kvs = []
                for g in range(BC // 128):
                    kv = jnp.dot(t[g * 128:(g + 1) * 128, :], wb[2 * NB + r, :, g * 128:(g + 1) * 128],
                                 preferred_element_type=f32)
                    kvs.append(jnp.where(same_head, kv, 0.0).astype(bf16))
            if i == 2:
                ms = []
                for g in range(BC // 128):
                    go = pl.multiple_of(r * BC + g * 128, 128)
                    ms.append(jnp.dot(kvs[g], wob[pl.ds(go, 128), :], preferred_element_type=f32).astype(bf16))
                m_r = jnp.concatenate(ms, axis=0)
        vpu_scores(kf_s, sx_s, kbs, pieces[SEG:], link2, True)
        for i in range(nh):
            y = bacc[i * hw:(i + 1) * hw, :] + jnp.dot(a_rows[i], m_r, preferred_element_type=f32)
            bacc[i * hw:(i + 1) * hw, :] = y
            ob_st[i * hw:(i + 1) * hw, :] = y.astype(bf16)
        return carry

    lax.fori_loop(0, NB, b_body, 0)
    out_copy(ob_st, 0, S, D)

    a_sl = slots(UN, NC + SK)
    c_sl = slots(UN, 0)

    def att_body(i, carry):
        m0, mp, _ = carry
        mk_, mp = run(i * (UN // G), a_sl, c_sl, {0: m0}, mp)
        return mk_[UN], mp, (i + 1) * (UN // G)

    n_it = (NU - UT) // UN
    assert n_it * UN + UT == NU and UN % G == 0 and UT % G == 0
    m_last, mp_last, g_last = lax.fori_loop(0, n_it, att_body, (mk[0], mp0, jnp.int32(0)))

    o_rows = []
    first_free = UT * NC - (NC + SK)

    def extra(t):
        k = t - first_free
        if k in (0, 4):
            if k == 0:
                o_rows.append(ot_s[0].T)
            c0 = (k // 4) * (D // 2)
            y = jnp.dot(o_rows[0], woa[:, c0:c0 + D // 2], preferred_element_type=f32)
            oa_st[0:TQ, c0:c0 + D // 2] = y.astype(bf16)
        if k == 3:
            o_rows.append(ot_s[1].T)

    a_tail = [a if a[0] < UT else None for a in slots(UT, NC + SK)]
    run(g_last, a_tail, slots(UT, 0), {0: m_last}, mp_last, extra=extra)
    out_copy(oa_st, 0, TQ, 0)

    oa_st[TQ:2 * TQ, :] = jnp.dot(o_rows[1], woa[...], preferred_element_type=f32).astype(bf16)
    out_copy(oa_st, TQ, TQ, 0)
    oa_st[2 * TQ:3 * TQ, :] = lax.dot_general(ot_s[2], woa[...], TN, preferred_element_type=f32).astype(bf16)
    out_copy(oa_st, 2 * TQ, TQ, 0)
    o_last = ot_s[3].T
    for p0, pn in OA_LAST:
        y = jnp.dot(o_last[p0:p0 + pn], woa[...], preferred_element_type=f32)
        oa_st[3 * TQ + p0:3 * TQ + p0 + pn, :] = y.astype(bf16)
        out_copy(oa_st, 3 * TQ + p0, pn, 0)

    wait(g_out)


@jax.jit
def pallas_concat_heads__mha_block__linear_attn_block__prompt_kernel(
    A_x: jax.Array,
    A_wqkv: jax.Array,
    A_wo: jax.Array,
    B_x: jax.Array,
    B_wqkv: jax.Array,
    B_wo: jax.Array,
):
    assert A_x.shape == (1, S, D) and B_x.shape == (1, S, D)
    any_spec = pl.BlockSpec(memory_space=pl.ANY)
    out = pl.pallas_call(
        _kernel,
        out_shape=jax.ShapeDtypeStruct((S, 2 * D), bf16),
        in_specs=[any_spec] * 6,
        out_specs=any_spec,
        scratch_shapes=[
            pltpu.VMEM((S, D), bf16),
            pltpu.VMEM((D, 3 * D), bf16),
            pltpu.VMEM((D, D), bf16),
            pltpu.VMEM((S, D), bf16),
            pltpu.VMEM((3 * NB, D, BC), bf16),
            pltpu.VMEM((D, D), bf16),
            pltpu.VMEM((NG, S, 128), bf16),
            pltpu.VMEM((NQ, D, TQ), bf16),
            pltpu.VMEM((D, S), bf16),
            pltpu.VMEM((NQ, D, TQ), bf16),
            pltpu.VMEM((S, TQ), f32),
            pltpu.VMEM((S, TQ), f32),
            pltpu.VMEM((S, D), f32),
            pltpu.VMEM((S, D), bf16),
            pltpu.VMEM((S, D), bf16),
            pltpu.VMEM((NU, NKV, TQ), f32),
            pltpu.VMEM((8, 128), f32),
            pltpu.VMEM((NQ, D, TQ), f32),
            pltpu.VMEM((NG, NKV, 128), f32),
            pltpu.VMEM((NQ * NG * 3, NKV, TQ), f32),
            pltpu.VMEM((NG, NKV, 128), f32),
            pltpu.SemaphoreType.DMA((N_SEM,)),
        ],
        compiler_params=pltpu.CompilerParams(vmem_limit_bytes=120 * 1024 * 1024),
    )(A_x.reshape(S, D), A_wqkv, A_wo, B_x.reshape(S, D), B_wqkv, B_wo)
    return out.reshape(1, S, 2 * D)
```

```python
import math

import jax
import jax.numpy as jnp
from jax import lax
import jax.experimental.pallas as pl
import jax.experimental.pallas.tpu as pltpu

f32 = jnp.float32
bf16 = jnp.bfloat16

S = 2048
D = 1024
H = 32
DH = D // H
G = 128 // DH
NG = D // 128

TQ = 512
CK = 256
SUB = 16
SK = 1
UN = 12
UT = 8
NQ = S // TQ
NU = H * NQ
NC = S // CK
NS = CK // SUB

NKV = 32
CX, CX2 = 1, 3
X0, X2 = CX * CK, CX2 * CK
SEG = 100


def _second(gidx, hh):
    return hh >= 2 or (hh == 1 and gidx % (UN // G) < 2)


BC = 256
NB = D // BC
HB = BC // DH

NT = (((1,), (1,)), ((), ()))
TN = (((0,), (0,)), ((), ()))

QSCALE = (DH ** -0.5) * math.log2(math.e)

K_CH = [(0, 128), (128, 128), (256, 256), (512, 256), (768, 256)]
XH = 1024
OA_LAST = [(0, 256), (256, 128), (384, 64), (448, 64)]
N_SEM = len(K_CH) + 3


def _phi(t):
    return jnp.where(t > 0, t + 1.0, jnp.exp(t)) + 1e-6


def _kernel(xa_hbm, wa_hbm, woa_hbm, xb_hbm, wb_hbm, wob_hbm, out_hbm,
            xa, wa, woa, xb, wb, wob,
            k_s, qt_s, vt_s, ot_s, sa, sb, bacc, oa_st, ob_st, sx_s, one_s, qf_s, kf_s, sx2_s, kf2_s, sem):
    groups = [[] for _ in range(N_SEM)]

    def copy(grp, src, dst):
        cp = pltpu.make_async_copy(src, dst, sem.at[grp])
        groups[grp].append(cp)
        cp.start()

    def wait(grp):
        for cp in groups[grp]:
            cp.wait()

    g_qv, g_b, g_out = len(K_CH), len(K_CH) + 1, len(K_CH) + 2
    for i, (k, n) in enumerate(K_CH):
        copy(i, xa_hbm.at[pl.ds(0, XH), pl.ds(k, n)], xa.at[pl.ds(0, XH), pl.ds(k, n)])
        copy(i, wa_hbm.at[pl.ds(k, n), pl.ds(D, D)], wa.at[pl.ds(k, n), pl.ds(D, D)])
    copy(len(K_CH) - 1, xa_hbm.at[pl.ds(XH, 512), :], xa.at[pl.ds(XH, 512), :])
    copy(g_qv, xa_hbm.at[pl.ds(XH + 512, 512), :], xa.at[pl.ds(XH + 512, 512), :])
    copy(g_qv, wa_hbm.at[:, pl.ds(0, D)], wa.at[:, pl.ds(0, D)])
    copy(g_qv, wa_hbm.at[:, pl.ds(2 * D, D)], wa.at[:, pl.ds(2 * D, D)])
    copy(g_b, xb_hbm, xb)
    for j in range(3 * NB):
        copy(g_b, wb_hbm.at[:, pl.ds(j * BC, BC)], wb.at[j])
    copy(g_b, wob_hbm, wob)
    copy(g_b, woa_hbm, woa)

    def out_copy(st, r0, n, col):
        copy(g_out, st.at[pl.ds(r0, n), :], out_hbm.at[pl.ds(r0, n), pl.ds(col, D)])

    def k_store(r0, r1, y):
        yb = y.astype(bf16)
        for g in range(NG):
            k_s[g, r0:r1, :] = yb[:, g * 128:(g + 1) * 128]
            if r0 <= X0 < r1:
                kf_s[g] = y[X0 - r0:X0 - r0 + NKV, g * 128:(g + 1) * 128]
            if r0 <= X2 < r1:
                kf2_s[g] = y[X2 - r0:X2 - r0 + NKV, g * 128:(g + 1) * 128]

    def kproj(r0, r1):
        k_store(r0, r1, jnp.dot(xa[r0:r1, :], wa[:, D:2 * D], preferred_element_type=f32))

    def zero_body(i, carry):
        bacc[pl.ds(pl.multiple_of(i * 128, 128), 128), :] = jnp.zeros((128, D), f32)
        return carry

    lax.fori_loop(0, S // 128, zero_body, 0)
    one_s[...] = jnp.ones_like(one_s)
    for i, (k, n) in enumerate(K_CH):
        wait(i)
        y = jnp.dot(xa[0:XH, k:k + n], wa[k:k + n, D:2 * D], preferred_element_type=f32)
        if i > 0:
            y = y + jnp.concatenate([sa[0:XH, :], sa[XH:2 * XH, :]], axis=1)
        if i < len(K_CH) - 1:
            sa[0:XH, :] = y[:, 0:TQ]
            sa[XH:2 * XH, :] = y[:, TQ:2 * TQ]
        else:
            k_store(0, XH, y)
    kproj(XH, XH + 512)
    wait(g_qv)
    kproj(XH + 512, S)

    ng = NKV // 8

    def vpu_scores(kf, sx, kbs, todo, link, slow):
        always = one_s[...] > 0.0
        always2 = one_s[...] > 0.5
        fin = None
        for grp, hh, row0, qi, q0, dst in todo:
            if hh not in kbs:
                k32 = kf[grp]
                l0 = (hh % G) * DH
                kbs[hh] = [jnp.broadcast_to(k32[:, l0 + d:l0 + d + 1], (NKV, 128)) for d in range(DH)]
            q32 = qf_s[qi, pl.ds(row0, DH), q0:q0 + 128]
            acc = None
            for d in range(DH):
                qd = jnp.broadcast_to(q32[d:d + 1, :], (8, 128))
                if fin is not None and 1 <= d < ng:
                    gf = (DH - 1 + d) % ng
                    qd = lax.select(always, qd, fin[gf * 8:(gf + 1) * 8])
                elif link is not None:
                    qd = lax.select(always, qd, link)
                if slow and link is not None:
                    qd = lax.select(always2, qd, link)
                t_ = kbs[hh][d] * jnp.concatenate([qd] * ng, axis=0)
                acc = t_ if acc is None else acc + t_
                link = acc[(d % ng) * 8:(d % ng + 1) * 8]
            sx[dst, :, q0:q0 + 128] = acc
            fin = acc
        return fin

    WC = 512
    XR = S // 2

    def proj_t(wcol):
        wt = wa[:, wcol:wcol + WC].T
        return [lax.dot_general(wt, xa[i * XR:(i + 1) * XR, :], NT, preferred_element_type=f32)
                for i in range(S // XR)]

    for co in range(0, D, WC):
        for i, y in enumerate(proj_t(co)):
            ys = y * QSCALE
            yb = ys.astype(bf16)
            for q in range(XR // TQ):
                qf_s[i * (XR // TQ) + q, co:co + WC, :] = ys[:, q * TQ:(q + 1) * TQ]
                qt_s[i * (XR // TQ) + q, co:co + WC, :] = yb[:, q * TQ:(q + 1) * TQ]
    vpu_scores(kf2_s, sx2_s, {},
               [(g, g * G + hh, (g * G + hh) * DH, qi, q0, (qi * NG + g) * 3 + hh - 1)
                for g0 in range(0, NG, WC // 128) for qi in range(NQ) for g in range(g0, g0 + WC // 128)
                for hh in range(1, G) if _second(qi * NG + g, hh) for q0 in range(0, TQ, 128)],
               None, True)
    for co in range(0, D, WC):
        for i, y in enumerate(proj_t(2 * D + co)):
            vt_s[co:co + WC, i * XR:(i + 1) * XR] = y.astype(bf16)

    bufs = (sa, sb)

    def offsets(gidx):
        if isinstance(gidx, int):
            return (gidx % NG) * 128, gidx % NG, gidx // NG
        gb = gidx & (NG - 1)
        return pl.multiple_of(gb * 128, 128), gb, lax.shift_right_logical(gidx, NG.bit_length() - 1)

    def run(g0, a_slots, c_slots, m_known, mp, extra=None, use_sx=True):
        offs = {}

        def off(u):
            if u // G not in offs:
                offs[u // G] = offsets(g0 + u // G)
            return offs[u // G]

        qms = {}
        prev_mh = None
        acc = None
        lhist = []
        for t, (a, cc) in enumerate(zip(a_slots, c_slots)):
            mh = None
            if a is not None:
                ua, c = a
                fb, gb, qi = off(ua)
                if ua not in qms:
                    hh = ua % G
                    qh = qt_s[qi, pl.ds(fb + hh * DH, DH), :]
                    parts = []
                    if hh > 0:
                        parts.append(jnp.zeros((hh * DH, TQ), bf16))
                    parts.append(qh)
                    if hh < G - 1:
                        parts.append(jnp.zeros(((G - 1 - hh) * DH, TQ), bf16))
                    qms[ua] = jnp.concatenate(parts, axis=0)
                if use_sx and c == CX:
                    kg = k_s[gb, X0 + NKV:(c + 1) * CK, :]
                    s = jnp.concatenate([sx_s[qi * H + gb * G + ua % G],
                                         jnp.dot(kg, qms[ua], preferred_element_type=f32)], axis=0)
                elif use_sx and c == CX2 and _second(ua // G, ua % G):
                    kg = k_s[gb, X2 + NKV:(c + 1) * CK, :]
                    s = jnp.concatenate([sx2_s[(qi * NG + gb) * 3 + ua % G - 1],
                                         jnp.dot(kg, qms[ua], preferred_element_type=f32)], axis=0)
                else:
                    kg = k_s[gb, c * CK:(c + 1) * CK, :]
                    s = jnp.dot(kg, qms[ua], preferred_element_type=f32)
                bufs[ua % 2][c * CK:(c + 1) * CK, :] = s
                mh = []
                for j in range(NS):
                    sm = jnp.max(s[j * SUB:(j + 1) * SUB].reshape(SUB // 8, 8, TQ), axis=0)
                    mp = sm if (c == 0 and j == 0) else jnp.maximum(mp, sm)
                    mh.append(mp)
                if c == NC - 1:
                    m_known[ua] = jnp.max(mp, axis=0, keepdims=True)
            elif extra is not None:
                extra(t)
            if cc is not None:
                uc, c = cc
                fb, gb, qi = off(uc)
                ho = fb + (uc % G) * DH
                s_c = bufs[uc % 2]
                m_c = m_known[uc]
                if c == 0:
                    lhist = []
                ps_ = []
                for j in range(NS):
                    g = c * NS + j
                    r0 = c * CK + j * SUB
                    d0 = s_c[r0:r0 + 8, :] - m_c
                    if g >= 1:
                        d0 = jnp.minimum(d0, lhist[g - 1])
                    if prev_mh is not None and j % 2 == 1:
                        d0 = jnp.minimum(d0, jnp.abs(prev_mh[j]))
                    d1 = s_c[r0 + 8:r0 + SUB, :] - m_c
                    p = jnp.exp2(jnp.concatenate([d0, d1], axis=0))
                    ps = jnp.sum(p.reshape(SUB // 8, 8, TQ), axis=0)
                    lhist.append(ps if g == 0 else lhist[-1] + ps)
                    ps_.append(p)
                pb = jnp.concatenate(ps_, axis=0).astype(bf16)
                vt = vt_s[pl.ds(ho, DH), c * CK:(c + 1) * CK]
                o = jnp.dot(vt, pb, preferred_element_type=f32)
                acc = o if c == 0 else acc + o
                if c == NC - 1:
                    l = jnp.sum(lhist[-1], axis=0, keepdims=True)
                    ot_s[qi, pl.ds(ho, DH), :] = (acc * (1.0 / l)).astype(bf16)
            prev_mh = mh
        return m_known, mp

    def slots(n_units, lead):
        return [((t + lead) // NC, (t + lead) % NC) for t in range(n_units * NC)]

    a0 = slots(2, 0)[:NC + SK]
    mk, mp0 = run(0, a0, [None] * len(a0), {}, None, use_sx=False)

    wait(g_b)
    same_head = (lax.broadcasted_iota(jnp.int32, (128, 128), 0) // DH
                 == lax.broadcasted_iota(jnp.int32, (128, 128), 1) // DH)

    def b_body(r, carry):
        co = pl.multiple_of(r * BC, BC)
        always = one_s[...] > 0.0
        pieces = [(r * (BC // 128) + hh // G, hh, co + hh * DH, qi, q0, qi * H + r * HB + hh)
                  for hh in range(HB) for qi in range(NQ) for q0 in range(0, TQ, 128)]
        kbs = {}
        link1 = vpu_scores(kf_s, sx_s, kbs, pieces[:SEG], None, False)
        pk = _phi(jnp.dot(xb[...], wb[NB + r], preferred_element_type=f32))
        z8 = jnp.sum(pk.reshape(S // 8, 8, BC), axis=0)
        z = jnp.sum(z8.T, axis=1, keepdims=True)
        t = jnp.dot(pk.astype(bf16).T, xb[...], preferred_element_type=f32).astype(bf16)
        w32 = wb[r].astype(f32)
        w00 = jnp.where(jnp.concatenate([always] * ng, axis=0), w32[0:NKV, 0:128], link1)
        w32 = jnp.concatenate([jnp.concatenate([w00, w32[0:NKV, 128:]], axis=1), w32[NKV:]], axis=0)
        wqt = w32.T.astype(bf16)
        nh = 4
        hw = S // nh
        a_rows = []
        for i in range(nh):
            pqt = _phi(lax.dot_general(wqt, xb[i * hw:(i + 1) * hw, :], NT, preferred_element_type=f32))
            den = jnp.sum((pqt * z).reshape(HB, DH, hw), axis=1, keepdims=True) + 1e-6
            at = pqt.reshape(HB, DH, hw) * (1.0 / den)
            a_rows.append(at.reshape(BC, hw).T.astype(bf16))
            if i == nh - 1:
                link2 = at.reshape(BC, hw)[BC - 8:BC, hw - 128:hw]
            if i == 1:
                kvs = []
                for g in range(BC // 128):
                    kv = jnp.dot(t[g * 128:(g + 1) * 128, :], wb[2 * NB + r, :, g * 128:(g + 1) * 128],
                                 preferred_element_type=f32)
                    kvs.append(jnp.where(same_head, kv, 0.0).astype(bf16))
            if i == 2:
                ms = []
                for g in range(BC // 128):
                    go = pl.multiple_of(r * BC + g * 128, 128)
                    ms.append(jnp.dot(kvs[g], wob[pl.ds(go, 128), :], preferred_element_type=f32).astype(bf16))
                m_r = jnp.concatenate(ms, axis=0)
        vpu_scores(kf_s, sx_s, kbs, pieces[SEG:], link2, True)
        for i in range(nh):
            y = bacc[i * hw:(i + 1) * hw, :] + jnp.dot(a_rows[i], m_r, preferred_element_type=f32)
            bacc[i * hw:(i + 1) * hw, :] = y
            ob_st[i * hw:(i + 1) * hw, :] = y.astype(bf16)
        return carry

    lax.fori_loop(0, NB, b_body, 0)
    out_copy(ob_st, 0, S, D)

    a_sl = slots(UN, NC + SK)
    c_sl = slots(UN, 0)

    def att_body(i, carry):
        m0, mp, _ = carry
        mk_, mp = run(i * (UN // G), a_sl, c_sl, {0: m0}, mp)
        return mk_[UN], mp, (i + 1) * (UN // G)

    n_it = (NU - UT) // UN
    assert n_it * UN + UT == NU and UN % G == 0 and UT % G == 0
    m_last, mp_last, g_last = lax.fori_loop(0, n_it, att_body, (mk[0], mp0, jnp.int32(0)))

    o_rows = []
    first_free = UT * NC - (NC + SK)

    def extra(t):
        k = t - first_free
        if k in (0, 4):
            if k == 0:
                o_rows.append(ot_s[0].T)
            c0 = (k // 4) * (D // 2)
            y = jnp.dot(o_rows[0], woa[:, c0:c0 + D // 2], preferred_element_type=f32)
            oa_st[0:TQ, c0:c0 + D // 2] = y.astype(bf16)
        if k == 3:
            o_rows.append(ot_s[1].T)

    a_tail = [a if a[0] < UT else None for a in slots(UT, NC + SK)]
    run(g_last, a_tail, slots(UT, 0), {0: m_last}, mp_last, extra=extra)
    out_copy(oa_st, 0, TQ, 0)

    oa_st[TQ:2 * TQ, :] = jnp.dot(o_rows[1], woa[...], preferred_element_type=f32).astype(bf16)
    out_copy(oa_st, TQ, TQ, 0)
    oa_st[2 * TQ:3 * TQ, :] = lax.dot_general(ot_s[2], woa[...], TN, preferred_element_type=f32).astype(bf16)
    out_copy(oa_st, 2 * TQ, TQ, 0)
    o_last = ot_s[3].T
    for p0, pn in OA_LAST:
        y = jnp.dot(o_last[p0:p0 + pn], woa[...], preferred_element_type=f32)
        oa_st[3 * TQ + p0:3 * TQ + p0 + pn, :] = y.astype(bf16)
        out_copy(oa_st, 3 * TQ + p0, pn, 0)

    wait(g_out)


@jax.jit
def pallas_concat_heads__mha_block__linear_attn_block__prompt_kernel(
    A_x: jax.Array,
    A_wqkv: jax.Array,
    A_wo: jax.Array,
    B_x: jax.Array,
    B_wqkv: jax.Array,
    B_wo: jax.Array,
):
    assert A_x.shape == (1, S, D) and B_x.shape == (1, S, D)
    any_spec = pl.BlockSpec(memory_space=pl.ANY)
    out = pl.pallas_call(
        _kernel,
        out_shape=jax.ShapeDtypeStruct((S, 2 * D), bf16),
        in_specs=[any_spec] * 6,
        out_specs=any_spec,
        scratch_shapes=[
            pltpu.VMEM((S, D), bf16),
            pltpu.VMEM((D, 3 * D), bf16),
            pltpu.VMEM((D, D), bf16),
            pltpu.VMEM((S, D), bf16),
            pltpu.VMEM((3 * NB, D, BC), bf16),
            pltpu.VMEM((D, D), bf16),
            pltpu.VMEM((NG, S, 128), bf16),
            pltpu.VMEM((NQ, D, TQ), bf16),
            pltpu.VMEM((D, S), bf16),
            pltpu.VMEM((NQ, D, TQ), bf16),
            pltpu.VMEM((S, TQ), f32),
            pltpu.VMEM((S, TQ), f32),
            pltpu.VMEM((S, D), f32),
            pltpu.VMEM((S, D), bf16),
            pltpu.VMEM((S, D), bf16),
            pltpu.VMEM((NU, NKV, TQ), f32),
            pltpu.VMEM((8, 128), f32),
            pltpu.VMEM((NQ, D, TQ), f32),
            pltpu.VMEM((NG, NKV, 128), f32),
            pltpu.VMEM((NQ * NG * 3, NKV, TQ), f32),
            pltpu.VMEM((NG, NKV, 128), f32),
            pltpu.SemaphoreType.DMA((N_SEM,)),
        ],
        compiler_params=pltpu.CompilerParams(vmem_limit_bytes=120 * 1024 * 1024),
    )(A_x.reshape(S, D), A_wqkv, A_wo, B_x.reshape(S, D), B_wqkv, B_wo)
    return out.reshape(1, S, 2 * D)
```

```python
import math

import jax
import jax.numpy as jnp
from jax import lax
import jax.experimental.pallas as pl
import jax.experimental.pallas.tpu as pltpu

f32 = jnp.float32
bf16 = jnp.bfloat16

S = 2048
D = 1024
H = 32
DH = D // H
G = 128 // DH
NG = D // 128

TQ = 512
CK = 256
SUB = 16
SK = 1
UN = 12
UT = 8
NQ = S // TQ
NU = H * NQ
NC = S // CK
NS = CK // SUB

NKV = 32
CX, CX2 = 1, 3
X0, X2 = CX * CK, CX2 * CK
SEG = 100


def _second(gidx, hh):
    return hh >= 2 or (hh == 1 and gidx % (UN // G) < 2)


BC = 256
NB = D // BC
HB = BC // DH

NT = (((1,), (1,)), ((), ()))
TN = (((0,), (0,)), ((), ()))

QSCALE = (DH ** -0.5) * math.log2(math.e)

K_CH = [(0, 128), (128, 128), (256, 256), (512, 256), (768, 256)]
XH = 1024
OA_LAST = [(0, 256), (256, 128), (384, 64), (448, 64)]
N_SEM = len(K_CH) + 4


def _phi(t):
    return jnp.where(t > 0, t + 1.0, jnp.exp(t)) + 1e-6


def _kernel(xa_hbm, wa_hbm, woa_hbm, xb_hbm, wb_hbm, wob_hbm, out_hbm,
            xa, wa, woa, xb, wb, wob,
            k_s, qt_s, vt_s, ot_s, sa, sb, bacc, oa_st, ob_st, sx_s, one_s, qf_s, kf_s, sx2_s, kf2_s, sem):
    groups = [[] for _ in range(N_SEM)]

    def copy(grp, src, dst):
        cp = pltpu.make_async_copy(src, dst, sem.at[grp])
        groups[grp].append(cp)
        cp.start()

    def wait(grp):
        for cp in groups[grp]:
            cp.wait()

    g_qv, g_b, g_out = len(K_CH), len(K_CH) + 1, len(K_CH) + 2
    g_first = len(K_CH) + 3
    HX = XH // 2
    for i, (k, n) in enumerate(K_CH):
        if i == 0:
            for grp, o in ((g_first, 0), (0, 1)):
                copy(grp, xa_hbm.at[pl.ds(o * HX, HX), pl.ds(k, n)], xa.at[pl.ds(o * HX, HX), pl.ds(k, n)])
                copy(grp, wa_hbm.at[pl.ds(k, n), pl.ds(D + o * TQ, TQ)], wa.at[pl.ds(k, n), pl.ds(D + o * TQ, TQ)])
            continue
        copy(i, xa_hbm.at[pl.ds(0, XH), pl.ds(k, n)], xa.at[pl.ds(0, XH), pl.ds(k, n)])
        copy(i, wa_hbm.at[pl.ds(k, n), pl.ds(D, D)], wa.at[pl.ds(k, n), pl.ds(D, D)])
    copy(len(K_CH) - 1, xa_hbm.at[pl.ds(XH, 512), :], xa.at[pl.ds(XH, 512), :])
    copy(g_qv, xa_hbm.at[pl.ds(XH + 512, 512), :], xa.at[pl.ds(XH + 512, 512), :])
    copy(g_qv, wa_hbm.at[:, pl.ds(0, D)], wa.at[:, pl.ds(0, D)])
    copy(g_qv, wa_hbm.at[:, pl.ds(2 * D, D)], wa.at[:, pl.ds(2 * D, D)])
    copy(g_b, xb_hbm, xb)
    for j in range(3 * NB):
        copy(g_b, wb_hbm.at[:, pl.ds(j * BC, BC)], wb.at[j])
    copy(g_b, wob_hbm, wob)
    copy(g_b, woa_hbm, woa)

    def out_copy(st, r0, n, col):
        copy(g_out, st.at[pl.ds(r0, n), :], out_hbm.at[pl.ds(r0, n), pl.ds(col, D)])

    def k_store(r0, r1, y):
        yb = y.astype(bf16)
        for g in range(NG):
            k_s[g, r0:r1, :] = yb[:, g * 128:(g + 1) * 128]
            if r0 <= X0 < r1:
                kf_s[g] = y[X0 - r0:X0 - r0 + NKV, g * 128:(g + 1) * 128]
            if r0 <= X2 < r1:
                kf2_s[g] = y[X2 - r0:X2 - r0 + NKV, g * 128:(g + 1) * 128]

    def kproj(r0, r1):
        k_store(r0, r1, jnp.dot(xa[r0:r1, :], wa[:, D:2 * D], preferred_element_type=f32))

    one_s[...] = jnp.ones_like(one_s)
    n0 = K_CH[0][1]
    wait(g_first)
    sa[0:HX, :] = jnp.dot(xa[0:HX, 0:n0], wa[0:n0, D:D + TQ], preferred_element_type=f32)
    wait(0)
    sa[HX:XH, :] = jnp.dot(xa[HX:XH, 0:n0], wa[0:n0, D:D + TQ], preferred_element_type=f32)
    sa[XH:2 * XH, :] = jnp.dot(xa[0:XH, 0:n0], wa[0:n0, D + TQ:2 * D], preferred_element_type=f32)
    for i, (k, n) in enumerate(K_CH):
        if i == 0:
            continue
        wait(i)
        y = jnp.dot(xa[0:XH, k:k + n], wa[k:k + n, D:2 * D], preferred_element_type=f32)
        if i > 0:
            y = y + jnp.concatenate([sa[0:XH, :], sa[XH:2 * XH, :]], axis=1)
        if i < len(K_CH) - 1:
            sa[0:XH, :] = y[:, 0:TQ]
            sa[XH:2 * XH, :] = y[:, TQ:2 * TQ]
        else:
            k_store(0, XH, y)
    kproj(XH, XH + 512)
    wait(g_qv)
    kproj(XH + 512, S)

    ng = NKV // 8

    def vpu_scores(kf, sx, kbs, todo, link, slow):
        always = one_s[...] > 0.0
        always2 = one_s[...] > 0.5
        fin = None
        for grp, hh, row0, qi, q0, dst in todo:
            if hh not in kbs:
                k32 = kf[grp]
                l0 = (hh % G) * DH
                kbs[hh] = [jnp.broadcast_to(k32[:, l0 + d:l0 + d + 1], (NKV, 128)) for d in range(DH)]
            q32 = qf_s[qi, pl.ds(row0, DH), q0:q0 + 128]
            acc = None
            for d in range(DH):
                qd = jnp.broadcast_to(q32[d:d + 1, :], (8, 128))
                if fin is not None and 1 <= d < ng:
                    gf = (DH - 1 + d) % ng
                    qd = lax.select(always, qd, fin[gf * 8:(gf + 1) * 8])
                elif link is not None:
                    qd = lax.select(always, qd, link)
                if slow and link is not None:
                    qd = lax.select(always2, qd, link)
                t_ = kbs[hh][d] * jnp.concatenate([qd] * ng, axis=0)
                acc = t_ if acc is None else acc + t_
                link = acc[(d % ng) * 8:(d % ng + 1) * 8]
            sx[dst, :, q0:q0 + 128] = acc
            fin = acc
        return fin

    WC = 512
    XR = S // 2

    def proj_t(wcol):
        wt = wa[:, wcol:wcol + WC].T
        return [lax.dot_general(wt, xa[i * XR:(i + 1) * XR, :], NT, preferred_element_type=f32)
                for i in range(S // XR)]

    for co in range(0, D, WC):
        for i, y in enumerate(proj_t(co)):
            ys = y * QSCALE
            yb = ys.astype(bf16)
            for q in range(XR // TQ):
                qf_s[i * (XR // TQ) + q, co:co + WC, :] = ys[:, q * TQ:(q + 1) * TQ]
                qt_s[i * (XR // TQ) + q, co:co + WC, :] = yb[:, q * TQ:(q + 1) * TQ]
    vpu_scores(kf2_s, sx2_s, {},
               [(g, g * G + hh, (g * G + hh) * DH, qi, q0, (qi * NG + g) * 3 + hh - 1)
                for g0 in range(0, NG, WC // 128) for qi in range(NQ) for g in range(g0, g0 + WC // 128)
                for hh in range(1, G) if _second(qi * NG + g, hh) for q0 in range(0, TQ, 128)],
               None, True)
    for co in range(0, D, WC):
        for i, y in enumerate(proj_t(2 * D + co)):
            vt_s[co:co + WC, i * XR:(i + 1) * XR] = y.astype(bf16)

    bufs = (sa, sb)

    def offsets(gidx):
        if isinstance(gidx, int):
            return (gidx % NG) * 128, gidx % NG, gidx // NG
        gb = gidx & (NG - 1)
        return pl.multiple_of(gb * 128, 128), gb, lax.shift_right_logical(gidx, NG.bit_length() - 1)

    def run(g0, a_slots, c_slots, m_known, mp, extra=None, use_sx=True):
        offs = {}

        def off(u):
            if u // G not in offs:
                offs[u // G] = offsets(g0 + u // G)
            return offs[u // G]

        qms = {}
        prev_mh = None
        acc = None
        lhist = []
        for t, (a, cc) in enumerate(zip(a_slots, c_slots)):
            mh = None
            if a is not None:
                ua, c = a
                fb, gb, qi = off(ua)
                if ua not in qms:
                    hh = ua % G
                    qh = qt_s[qi, pl.ds(fb + hh * DH, DH), :]
                    parts = []
                    if hh > 0:
                        parts.append(jnp.zeros((hh * DH, TQ), bf16))
                    parts.append(qh)
                    if hh < G - 1:
                        parts.append(jnp.zeros(((G - 1 - hh) * DH, TQ), bf16))
                    qms[ua] = jnp.concatenate(parts, axis=0)
                if use_sx and c == CX:
                    kg = k_s[gb, X0 + NKV:(c + 1) * CK, :]
                    s = jnp.concatenate([sx_s[qi * H + gb * G + ua % G],
                                         jnp.dot(kg, qms[ua], preferred_element_type=f32)], axis=0)
                elif use_sx and c == CX2 and _second(ua // G, ua % G):
                    kg = k_s[gb, X2 + NKV:(c + 1) * CK, :]
                    s = jnp.concatenate([sx2_s[(qi * NG + gb) * 3 + ua % G - 1],
                                         jnp.dot(kg, qms[ua], preferred_element_type=f32)], axis=0)
                else:
                    kg = k_s[gb, c * CK:(c + 1) * CK, :]
                    s = jnp.dot(kg, qms[ua], preferred_element_type=f32)
                bufs[ua % 2][c * CK:(c + 1) * CK, :] = s
                mh = []
                for j in range(NS):
                    sm = jnp.max(s[j * SUB:(j + 1) * SUB].reshape(SUB // 8, 8, TQ), axis=0)
                    mp = sm if (c == 0 and j == 0) else jnp.maximum(mp, sm)
                    mh.append(mp)
                if c == NC - 1:
                    m_known[ua] = jnp.max(mp, axis=0, keepdims=True)
            elif extra is not None:
                extra(t)
            if cc is not None:
                uc, c = cc
                fb, gb, qi = off(uc)
                ho = fb + (uc % G) * DH
                s_c = bufs[uc % 2]
                m_c = m_known[uc]
                if c == 0:
                    lhist = []
                ps_ = []
                for j in range(NS):
                    g = c * NS + j
                    r0 = c * CK + j * SUB
                    d0 = s_c[r0:r0 + 8, :] - m_c
                    if g >= 1:
                        d0 = jnp.minimum(d0, lhist[g - 1])
                    if prev_mh is not None and j % 2 == 1:
                        d0 = jnp.minimum(d0, jnp.abs(prev_mh[j]))
                    d1 = s_c[r0 + 8:r0 + SUB, :] - m_c
                    p = jnp.exp2(jnp.concatenate([d0, d1], axis=0))
                    ps = jnp.sum(p.reshape(SUB // 8, 8, TQ), axis=0)
                    lhist.append(ps if g == 0 else lhist[-1] + ps)
                    ps_.append(p)
                pb = jnp.concatenate(ps_, axis=0).astype(bf16)
                vt = vt_s[pl.ds(ho, DH), c * CK:(c + 1) * CK]
                o = jnp.dot(vt, pb, preferred_element_type=f32)
                acc = o if c == 0 else acc + o
                if c == NC - 1:
                    l = jnp.sum(lhist[-1], axis=0, keepdims=True)
                    ot_s[qi, pl.ds(ho, DH), :] = (acc * (1.0 / l)).astype(bf16)
            prev_mh = mh
        return m_known, mp

    def slots(n_units, lead):
        return [((t + lead) // NC, (t + lead) % NC) for t in range(n_units * NC)]

    a0 = slots(2, 0)[:NC + SK]
    mk, mp0 = run(0, a0, [None] * len(a0), {}, None, use_sx=False)

    wait(g_b)
    same_head = (lax.broadcasted_iota(jnp.int32, (128, 128), 0) // DH
                 == lax.broadcasted_iota(jnp.int32, (128, 128), 1) // DH)

    def b_body(r, carry):
        co = pl.multiple_of(r * BC, BC)
        always = one_s[...] > 0.0
        pieces = [(r * (BC // 128) + hh // G, hh, co + hh * DH, qi, q0, qi * H + r * HB + hh)
                  for hh in range(HB) for qi in range(NQ) for q0 in range(0, TQ, 128)]
        kbs = {}
        link1 = vpu_scores(kf_s, sx_s, kbs, pieces[:SEG], None, False)
        pk = _phi(jnp.dot(xb[...], wb[NB + r], preferred_element_type=f32))
        z8 = jnp.sum(pk.reshape(S // 8, 8, BC), axis=0)
        z = jnp.sum(z8.T, axis=1, keepdims=True)
        t = jnp.dot(pk.astype(bf16).T, xb[...], preferred_element_type=f32).astype(bf16)
        w32 = wb[r].astype(f32)
        w00 = jnp.where(jnp.concatenate([always] * ng, axis=0), w32[0:NKV, 0:128], link1)
        w32 = jnp.concatenate([jnp.concatenate([w00, w32[0:NKV, 128:]], axis=1), w32[NKV:]], axis=0)
        wqt = w32.T.astype(bf16)
        nh = 4
        hw = S // nh
        a_rows = []
        for i in range(nh):
            pqt = _phi(lax.dot_general(wqt, xb[i * hw:(i + 1) * hw, :], NT, preferred_element_type=f32))
            den = jnp.sum((pqt * z).reshape(HB, DH, hw), axis=1, keepdims=True) + 1e-6
            at = pqt.reshape(HB, DH, hw) * (1.0 / den)
            a_rows.append(at.reshape(BC, hw).T.astype(bf16))
            if i == nh - 1:
                link2 = at.reshape(BC, hw)[BC - 8:BC, hw - 128:hw]
            if i == 1:
                kvs = []
                for g in range(BC // 128):
                    kv = jnp.dot(t[g * 128:(g + 1) * 128, :], wb[2 * NB + r, :, g * 128:(g + 1) * 128],
                                 preferred_element_type=f32)
                    kvs.append(jnp.where(same_head, kv, 0.0).astype(bf16))
            if i == 2:
                ms = []
                for g in range(BC // 128):
                    go = pl.multiple_of(r * BC + g * 128, 128)
                    ms.append(jnp.dot(kvs[g], wob[pl.ds(go, 128), :], preferred_element_type=f32).astype(bf16))
                m_r = jnp.concatenate(ms, axis=0)
        vpu_scores(kf_s, sx_s, kbs, pieces[SEG:], link2, True)
        for i in range(nh):
            prev = jnp.where(r > 0, bacc[i * hw:(i + 1) * hw, :], 0.0)
            y = prev + jnp.dot(a_rows[i], m_r, preferred_element_type=f32)
            bacc[i * hw:(i + 1) * hw, :] = y
            ob_st[i * hw:(i + 1) * hw, :] = y.astype(bf16)
        return carry

    lax.fori_loop(0, NB, b_body, 0)
    out_copy(ob_st, 0, S, D)

    a_sl = slots(UN, NC + SK)
    c_sl = slots(UN, 0)

    def att_body(i, carry):
        m0, mp, _ = carry
        mk_, mp = run(i * (UN // G), a_sl, c_sl, {0: m0}, mp)
        return mk_[UN], mp, (i + 1) * (UN // G)

    n_it = (NU - UT) // UN
    assert n_it * UN + UT == NU and UN % G == 0 and UT % G == 0
    m_last, mp_last, g_last = lax.fori_loop(0, n_it, att_body, (mk[0], mp0, jnp.int32(0)))

    o_rows = []
    first_free = UT * NC - (NC + SK)

    def extra(t):
        k = t - first_free
        if k in (0, 4):
            if k == 0:
                o_rows.append(ot_s[0].T)
            c0 = (k // 4) * (D // 2)
            y = jnp.dot(o_rows[0], woa[:, c0:c0 + D // 2], preferred_element_type=f32)
            oa_st[0:TQ, c0:c0 + D // 2] = y.astype(bf16)
        if k == 3:
            o_rows.append(ot_s[1].T)

    a_tail = [a if a[0] < UT else None for a in slots(UT, NC + SK)]
    run(g_last, a_tail, slots(UT, 0), {0: m_last}, mp_last, extra=extra)
    out_copy(oa_st, 0, TQ, 0)

    oa_st[TQ:2 * TQ, :] = jnp.dot(o_rows[1], woa[...], preferred_element_type=f32).astype(bf16)
    out_copy(oa_st, TQ, TQ, 0)
    oa_st[2 * TQ:3 * TQ, :] = lax.dot_general(ot_s[2], woa[...], TN, preferred_element_type=f32).astype(bf16)
    out_copy(oa_st, 2 * TQ, TQ, 0)
    o_last = ot_s[3].T
    for p0, pn in OA_LAST:
        y = jnp.dot(o_last[p0:p0 + pn], woa[...], preferred_element_type=f32)
        oa_st[3 * TQ + p0:3 * TQ + p0 + pn, :] = y.astype(bf16)
        out_copy(oa_st, 3 * TQ + p0, pn, 0)

    wait(g_out)


@jax.jit
def pallas_concat_heads__mha_block__linear_attn_block__prompt_kernel(
    A_x: jax.Array,
    A_wqkv: jax.Array,
    A_wo: jax.Array,
    B_x: jax.Array,
    B_wqkv: jax.Array,
    B_wo: jax.Array,
):
    assert A_x.shape == (1, S, D) and B_x.shape == (1, S, D)
    any_spec = pl.BlockSpec(memory_space=pl.ANY)
    out = pl.pallas_call(
        _kernel,
        out_shape=jax.ShapeDtypeStruct((S, 2 * D), bf16),
        in_specs=[any_spec] * 6,
        out_specs=any_spec,
        scratch_shapes=[
            pltpu.VMEM((S, D), bf16),
            pltpu.VMEM((D, 3 * D), bf16),
            pltpu.VMEM((D, D), bf16),
            pltpu.VMEM((S, D), bf16),
            pltpu.VMEM((3 * NB, D, BC), bf16),
            pltpu.VMEM((D, D), bf16),
            pltpu.VMEM((NG, S, 128), bf16),
            pltpu.VMEM((NQ, D, TQ), bf16),
            pltpu.VMEM((D, S), bf16),
            pltpu.VMEM((NQ, D, TQ), bf16),
            pltpu.VMEM((S, TQ), f32),
            pltpu.VMEM((S, TQ), f32),
            pltpu.VMEM((S, D), f32),
            pltpu.VMEM((S, D), bf16),
            pltpu.VMEM((S, D), bf16),
            pltpu.VMEM((NU, NKV, TQ), f32),
            pltpu.VMEM((8, 128), f32),
            pltpu.VMEM((NQ, D, TQ), f32),
            pltpu.VMEM((NG, NKV, 128), f32),
            pltpu.VMEM((NQ * NG * 3, NKV, TQ), f32),
            pltpu.VMEM((NG, NKV, 128), f32),
            pltpu.SemaphoreType.DMA((N_SEM,)),
        ],
        compiler_params=pltpu.CompilerParams(vmem_limit_bytes=120 * 1024 * 1024),
    )(A_x.reshape(S, D), A_wqkv, A_wo, B_x.reshape(S, D), B_wqkv, B_wo)
    return out.reshape(1, S, 2 * D)
```
